```python
import jax
import jax.numpy as jnp

def _softmax(x, axis=-1):
    return jax.nn.softmax(x, axis=axis)

def _gelu(x):
    return jax.nn.gelu(x, approximate=True)

def _silu(x):
    return jax.nn.silu(x)

def _sigmoid(x):
    return jax.nn.sigmoid(x)

def _layernorm(x, axis=-1, eps=1e-05):
    m = jnp.mean(x, axis=axis, keepdims=True)
    v = jnp.var(x, axis=axis, keepdims=True)
    return (x - m) / jnp.sqrt(v + eps)

def _scatter_add(tgt, idx, src, axis=0):
    return tgt.at[idx].add(src)

def _segment_sum(src, seg, n):
    return jax.ops.segment_sum(src, seg, n)

class _Rng:

    def __init__(self, key):
        self._k = key

    def _next(self):
        self._k, sub = jax.random.split(self._k)
        return sub

    def normal(self, shape):
        return jax.random.normal(self._next(), shape, dtype=jnp.bfloat16)

    def randint(self, lo, hi, shape):
        return jax.random.randint(self._next(), shape, lo, hi, dtype=jnp.int32)

    def uniform(self, shape, lo=0.0, hi=1.0):
        return jax.random.uniform(self._next(), shape, jnp.bfloat16, lo, hi)

    def permutation(self, n):
        return jax.random.permutation(self._next(), n)
kernel_name = 'adaLN_cond__compressed_kv_cla__mixer_s_mlp__decode'

def setup_inputs():
    _rng = _Rng(jax.random.key(int.from_bytes(__import__("os").urandom(4), "little")))
    _w = lambda a: (lambda t: t.astype(jnp.bfloat16) if jnp.issubdtype(t.dtype, jnp.floating) else t)(jnp.asarray(a))

    def _A_setup():
        B, H, Sq, Sk, D, M = (8, 32, 1, 4096, 128, 512)
        Dc = 4 * D
        return {'x': _w((lambda *s: _rng.normal(s) * 0.05)(B, Sq, M)), 'c_kv': _w((lambda *s: _rng.normal(s) * 0.05)(B, Sk, Dc)), 'w_q': _w((lambda *s: _rng.normal(s) * 0.05)(M, H, D) * M ** (-0.5)), 'w_uk': _w((lambda *s: _rng.normal(s) * 0.05)(Dc, H, D) * Dc ** (-0.5)), 'w_uv': _w((lambda *s: _rng.normal(s) * 0.05)(Dc, H, D) * Dc ** (-0.5)), 'w_o': _w((lambda *s: _rng.normal(s) * 0.05)(H, D, M) * (H * D) ** (-0.5))}
    _A_in = _A_setup()

    def _B_setup():
        B, S, D, F = (8, 1, 512, 1792)
        return {'x': _w((lambda *s: _rng.normal(s) * 0.05)(B, S, D)), 'w1': _w((lambda *s: _rng.normal(s) * 0.05)(D, D) * D ** (-0.5)), 'w2': _w((lambda *s: _rng.normal(s) * 0.05)(D, D) * D ** (-0.5)), 'w3': _w((lambda *s: _rng.normal(s) * 0.05)(D, F) * D ** (-0.5)), 'w4': _w((lambda *s: _rng.normal(s) * 0.05)(F, D) * F ** (-0.5))}
    _B_in = _B_setup()
    return {'A_x': _A_in['x'], 'A_c_kv': _A_in['c_kv'], 'A_w_q': _A_in['w_q'], 'A_w_uk': _A_in['w_uk'], 'A_w_uv': _A_in['w_uv'], 'A_w_o': _A_in['w_o'], 'B_x': _B_in['x'], 'B_w1': _B_in['w1'], 'B_w2': _B_in['w2'], 'B_w3': _B_in['w3'], 'B_w4': _B_in['w4'], 'c': _w((lambda *s: _rng.normal(s) * 0.05)(8, 512)), 'w_mod': _w((lambda *s: _rng.normal(s) * 0.05)(512, 6 * 512) * 512 ** (-0.5))}

def reference(A_x, A_c_kv, A_w_q, A_w_uk, A_w_uv, A_w_o, B_x, B_w1, B_w2, B_w3, B_w4, c, w_mod):

    def _A_ref(x, c_kv, w_q, w_uk, w_uv, w_o):
        B, Sq, M = (x.shape[0], x.shape[1], x.shape[2])
        Sk = c_kv.shape[1]
        H, D = (w_q.shape[1], w_q.shape[2])
        q = jnp.einsum('bqm,mhd->bhqd', x, w_q)
        k = jnp.einsum('bkc,chd->bhkd', c_kv, w_uk)
        v = jnp.einsum('bkc,chd->bhkd', c_kv, w_uv)
        scores = jnp.einsum('bhqd,bhkd->bhqk', q, k) * D ** (-0.5)
        off = Sk - Sq
        qi = jnp.arange(Sq)[:, None]
        kj = jnp.arange(Sk)[None, :]
        cmask = kj <= qi + off
        scores = jnp.where(cmask[None, None], scores, -1000000000.0)
        p = _softmax(scores, axis=-1)
        ctx = jnp.einsum('bhqk,bhkd->bhqd', p, v)
        return jnp.einsum('bhqd,hdm->bqm', ctx, w_o)

    def _B_ref(x, w1, w2, w3, w4):
        B, S, D = x.shape
        h = _gelu(_layernorm(x, axis=-1) @ w1)
        c = D // 4
        g0 = jnp.pad(h[:, :, 0 * c:1 * c], ((0, 0), (1, 0), (0, 0)))[:, :S, :]
        g1 = jnp.pad(h[:, :, 1 * c:2 * c], ((0, 0), (0, 1), (0, 0)))[:, 1:, :]
        g2 = jnp.pad(h[:, :, 2 * c:3 * c], ((0, 0), (2, 0), (0, 0)))[:, :S, :]
        g3 = jnp.pad(h[:, :, 3 * c:], ((0, 0), (0, 2), (0, 0)))[:, 2:, :]
        hs = jnp.concatenate([g0, g1, g2, g3], axis=-1) @ w2
        x1 = x + hs
        h2 = _gelu(_layernorm(x1, axis=-1) @ w3) @ w4
        return x1 + h2
    x = A_x
    mod = (_silu(c) @ w_mod).reshape(c.shape[0], 6, 1, -1)
    sa, ca, ga, sb, cb, gb = (mod[:, 0].copy(), mod[:, 1].copy(), mod[:, 2].copy(), mod[:, 3].copy(), mod[:, 4].copy(), mod[:, 5].copy())
    h = _layernorm(x, axis=-1) * (1 + ca) + sa
    x = x + ga * _A_ref(h, A_c_kv, A_w_q, A_w_uk, A_w_uv, A_w_o)
    h = _layernorm(x, axis=-1) * (1 + cb) + sb
    x = x + gb * _B_ref(h, B_w1, B_w2, B_w3, B_w4)
    return x
```

```python
import jax
import jax.numpy as jnp
from jax import lax
import jax.experimental.pallas as pl
import jax.experimental.pallas.tpu as pltpu

F32 = jnp.float32
BF16 = jnp.bfloat16
U32 = jnp.uint32
LANES = 128


def _layernorm(x, eps=1e-5):
    m = jnp.mean(x, axis=-1, keepdims=True)
    d = x - m
    v = jnp.mean(d * d, axis=-1, keepdims=True)
    return d * lax.rsqrt(v + eps)


def _dot(a, b):
    return jnp.dot(a, b, preferred_element_type=F32)


def _dot_nt(a, b):
    return lax.dot_general(a, b, (((1,), (1,)), ((), ())), preferred_element_type=F32)


def _head_pair(w_ref, j, rows, heads):
    u = w_ref
    a = u[pl.ds(j, rows // 2, stride=heads), :]
    b = u[pl.ds(j + heads // 2, rows // 2, stride=heads), :]
    lo = (a & U32(0xFFFF)) | (b << U32(16))
    hi = (a >> U32(16)) | (b & U32(0xFFFF0000))
    return pltpu.bitcast(lo, BF16), pltpu.bitcast(hi, BF16)


def _make_kernel(B, H, D, M, Dc, Sk, F):
    scale = float(D) ** -0.5
    KC = 512
    W4_CHUNKS = ((0, 896), (896, 640), (1536, 256))

    def kernel(x_hbm, ckv_hbm, wq_hbm, wuk_hbm, wuv_hbm, wo_hbm, w3_hbm, w4_hbm, c_hbm, wm_hbm,
               o_ref,
               x_v, ckv_v, wq_v, wuk_v, wuv_v, wo_v, w3_v, w4_v, c_v, wm_v,
               q_s, qa_s, s_s, ctx_s, cv_s, sems):
        n_sem = [0]

        def copy(src, dst):
            i = n_sem[0]
            n_sem[0] += 1
            return pltpu.make_async_copy(src, dst, sems.at[i])

        def cols(ref, c0, n):
            return ref.at[:, pl.ds(c0, n)]

        def rows(ref, r0, n):
            return ref.at[pl.ds(r0, n), :]

        ckv_cp = [copy(rows(ckv_hbm, b * Sk, Sk), rows(ckv_v, b * Sk, Sk)) for b in range(B)]
        c_cp = copy(c_hbm, c_v)
        x_cp = copy(x_hbm, x_v)
        wma_cp = copy(cols(wm_hbm, 0, 2 * M), cols(wm_v, 0, 2 * M))
        wq_cp = copy(wq_hbm.bitcast(U32), wq_v)
        wuk_cp = copy(wuk_hbm.bitcast(U32), wuk_v)
        wuv_cp = copy(wuv_hbm.bitcast(U32), wuv_v)
        wo_cp = copy(wo_hbm, wo_v)
        wmb_cp = copy(cols(wm_hbm, 2 * M, 4 * M), cols(wm_v, 2 * M, 4 * M))
        w3_cp = copy(w3_hbm, w3_v)
        w4_cp = [copy(rows(w4_hbm, r0, n), rows(w4_v, r0, n)) for r0, n in W4_CHUNKS]

        for cp in [c_cp, x_cp, wma_cp, wq_cp, wuk_cp, *ckv_cp, wuv_cp, wo_cp, wmb_cp, w3_cp, *w4_cp]:
            cp.start()

        c_cp.wait()
        c = c_v[...].astype(F32)
        sc = (c * jax.nn.sigmoid(c)).astype(BF16)
        x_cp.wait()
        x = x_v[...].astype(F32)
        xn = _layernorm(x)
        wma_cp.wait()
        mod_a = _dot(sc, wm_v[:, 0:2 * M])
        h = (xn * (1.0 + mod_a[:, M:2 * M]) + mod_a[:, 0:M]).astype(BF16)

        wq_cp.wait()

        def q_body(j, carry):
            w0, w1 = _head_pair(wq_v, j, M, H)
            q_s[2 * j] = _dot(h, w0)
            q_s[2 * j + 1] = _dot(h, w1)
            return carry

        lax.fori_loop(0, H // 2, q_body, 0)

        wuk_cp.wait()

        def qa_body(j, carry):
            ws = _head_pair(wuk_v, j, Dc, H)
            for p in range(2):
                r = _dot_nt(q_s[2 * j + p].astype(BF16), ws[p]) * scale
                for t in range(Dc // LANES):
                    qa_s[t, pl.ds(2 * j + p, B, stride=H), :] = r[:, t * LANES:(t + 1) * LANES]
            return carry

        lax.fori_loop(0, H // 2, qa_body, 0)

        def attn_body(b, carry):
            r0 = pl.multiple_of(b * H, H)
            k0 = pl.multiple_of(b * Sk, Sk)
            qb = jnp.concatenate(
                [qa_s[t, pl.ds(r0, H), :] for t in range(Dc // LANES)], axis=1).astype(BF16)
            pltpu.make_async_copy(rows(ckv_hbm, k0, Sk), rows(ckv_v, k0, Sk), sems.at[b]).wait()
            mt = None
            for i in range(Sk // KC):
                s = _dot_nt(qb, ckv_v[pl.ds(k0 + i * KC, KC), :])
                s_s[:, i * KC:(i + 1) * KC] = s
                for t in range(KC // LANES):
                    st = s[:, t * LANES:(t + 1) * LANES]
                    mt = st if mt is None else jnp.maximum(mt, st)
            m = jnp.max(mt, axis=1, keepdims=True)
            lt = None
            acc = None
            for i in range(Sk // KC):
                p = jnp.exp(s_s[:, i * KC:(i + 1) * KC] - m)
                for t in range(KC // LANES):
                    pt = p[:, t * LANES:(t + 1) * LANES]
                    lt = pt if lt is None else lt + pt
                d = _dot(p.astype(BF16), ckv_v[pl.ds(k0 + i * KC, KC), :])
                acc = d if acc is None else acc + d
            ctx = acc / jnp.sum(lt, axis=1, keepdims=True)
            for t in range(Dc // LANES):
                ctx_s[t, pl.ds(r0, H), :] = ctx[:, t * LANES:(t + 1) * LANES]
            return carry

        lax.fori_loop(0, B, attn_body, 0)

        wuv_cp.wait()

        def uv_body(j, carry):
            ws = _head_pair(wuv_v, j, Dc, H)
            for p in range(2):
                cx = jnp.concatenate(
                    [ctx_s[t, pl.ds(2 * j + p, B, stride=H), :] for t in range(Dc // LANES)],
                    axis=1).astype(BF16)
                cv_s[2 * j + p] = _dot(cx, ws[p])
            return carry

        lax.fori_loop(0, H // 2, uv_body, 0)

        cv = jnp.concatenate([cv_s[i] for i in range(H)], axis=1).astype(BF16)
        wo_cp.wait()
        att = _dot(cv, wo_v[...])
        wmb_cp.wait()
        mod_b = _dot(sc, wm_v[:, 2 * M:6 * M])
        ga, sb, cb, gb = (mod_b[:, i * M:(i + 1) * M] for i in range(4))
        x = x + ga * att
        h2 = _layernorm(x) * (1.0 + cb) + sb

        hn = _layernorm(h2).astype(BF16)
        w3_cp.wait()
        g = jax.nn.gelu(_dot(hn, w3_v[...]), approximate=True).astype(BF16)
        y = h2
        for cp, (f0, n) in zip(w4_cp, W4_CHUNKS):
            cp.wait()
            y = y + _dot(g[:, f0:f0 + n], w4_v[f0:f0 + n, :])
        o_ref[...] = (x + gb * y).astype(o_ref.dtype)

    return kernel


@jax.jit
def pallas_adaLN_cond__compressed_kv_cla__mixer_s_mlp__decode_kernel(
    A_x: jax.Array,
    A_c_kv: jax.Array,
    A_w_q: jax.Array,
    A_w_uk: jax.Array,
    A_w_uv: jax.Array,
    A_w_o: jax.Array,
    B_x: jax.Array,
    B_w1: jax.Array,
    B_w2: jax.Array,
    B_w3: jax.Array,
    B_w4: jax.Array,
    c: jax.Array,
    w_mod: jax.Array,
):
    B, Sq, M = A_x.shape
    _, Sk, Dc = A_c_kv.shape
    _, H, D = A_w_q.shape
    F = B_w3.shape[1]
    assert Sq == 1 and D == LANES

    ins = (
        A_x.reshape(B, M),
        A_c_kv.reshape(B * Sk, Dc),
        A_w_q.reshape(M * H, D),
        A_w_uk.reshape(Dc * H, D),
        A_w_uv.reshape(Dc * H, D),
        A_w_o.reshape(H * D, M),
        B_w3,
        B_w4,
        c,
        w_mod,
    )
    out = pl.pallas_call(
        _make_kernel(B, H, D, M, Dc, Sk, F),
        out_shape=jax.ShapeDtypeStruct((B, M), A_x.dtype),
        in_specs=[pl.BlockSpec(memory_space=pltpu.HBM)] * len(ins),
        out_specs=pl.BlockSpec(memory_space=pltpu.VMEM),
        scratch_shapes=[pltpu.VMEM((a.shape[0] // 2, D), U32) if i in (2, 3, 4) else pltpu.VMEM(a.shape, a.dtype) for i, a in enumerate(ins)] + [
            pltpu.VMEM((H, B, D), F32),
            pltpu.VMEM((Dc // LANES, B * H, LANES), F32),
            pltpu.VMEM((H, Sk), F32),
            pltpu.VMEM((Dc // LANES, B * H, LANES), F32),
            pltpu.VMEM((H, B, D), F32),
            pltpu.SemaphoreType.DMA((24,)),
        ],
        compiler_params=pltpu.CompilerParams(vmem_limit_bytes=100 * 1024 * 1024),
    )(*ins)
    return out.reshape(B, Sq, M)
```

```python
import jax
import jax.numpy as jnp
from jax import lax
import jax.experimental.pallas as pl
import jax.experimental.pallas.tpu as pltpu

F32 = jnp.float32
BF16 = jnp.bfloat16
U32 = jnp.uint32
LANES = 128

HI_BYTES = 49152
LO_BYTES = 49152
LAG = 32
KC = 512
ATTN_STEPS = 32
TAIL_STEPS = 20
W4_CUTS = (0, 1152, 1664, 1792)
NO_CHECKS = False


def _layernorm(x, eps=1e-5):
    m = jnp.mean(x, axis=-1, keepdims=True)
    d = x - m
    v = jnp.mean(d * d, axis=-1, keepdims=True)
    return d * lax.rsqrt(v + eps)


def _dot(a, b):
    return jnp.dot(a, b, preferred_element_type=F32)


def _dot_nt(a, b):
    return lax.dot_general(a, b, (((1,), (1,)), ((), ())), preferred_element_type=F32)


def _cut(start, total, piece):
    return [(start + o, min(piece, total - o)) for o in range(0, total, piece)]


class _Stream:
    def __init__(self):
        self.lo = []
        self.hi = []

    def add(self, src, dst, sem, row_bytes, base=0, rows=None):
        rows = src.shape[0] if rows is None else rows
        n_hi = max(8, HI_BYTES // row_bytes // 8 * 8)
        n_lo = max(8, LO_BYTES // row_bytes // 8 * 8)
        split = rows * n_hi // (n_hi + n_lo) // 8 * 8
        self.hi += [(src, dst, sem, base, o, n) for o, n in _cut(0, split, n_hi)]
        self.lo += [(src, dst, sem, base, o, n) for o, n in _cut(split, rows - split, n_lo)]

    @staticmethod
    def _start(item, priority):
        src, dst, sem, base, o, n = item
        r = pl.ds(base + o, n)
        pltpu.make_async_copy(src.at[r, :], dst.at[r, :], sem).start(priority=priority)

    def pump(self, steps=None):
        steps = len(self) if steps is None else steps
        for _ in range(steps):
            if self.lo:
                self._start(self.lo.pop(0), 1)
            if self.hi:
                self._start(self.hi.pop(0), 0)

    def __len__(self):
        return max(len(self.lo), len(self.hi))


def _spread(total, parts):
    return [total * (i + 1) // parts - total * i // parts for i in range(parts)]


def _make_kernel(B, H, D, M, Dc, Sk, F):
    scale = float(D) ** -0.5
    n_kc = Sk // KC
    n_ct = Dc // LANES

    def kernel(x_hbm, ckv_hbm, wq_hbm, wuk_hbm, wuv_hbm, wo_hbm, w3_hbm, w4_hbm, c_hbm, wm_hbm,
               o_ref,
               x_v, ckv_v, wq_v, wuk_v, wuv_v, wo_v, w3_v, w4_v, c_v, wm_v,
               wh_s, q_s, qa_s, s_s, ctx_s, cv_s, sems):
        wq_hbm, wuk_hbm, wuv_hbm = (w.bitcast(U32) for w in (wq_hbm, wuk_hbm, wuv_hbm))
        (sem_x, sem_c, sem_wm, sem_wq, sem_wuk, sem_wuv, sem_wo, sem_w3, *sem_w4) = (
            sems.at[B + i] for i in range(8 + len(W4_CUTS) - 1))

        def wait(src, dst, sem, r0=0, n=None):
            r = pl.ds(r0, src.shape[0] if n is None else n)
            pltpu.make_async_copy(src.at[r, :], dst.at[r, :], sem).wait()

        def split_heads(w_v, rows, stream, steps):
            pitch = rows // 2 + 1
            per_it = rows // 2 // len(steps)
            for it, n in enumerate(steps):
                def body(i, carry):
                    for t in range(8):
                        r = it * per_it + i * 8 + t
                        src = pl.multiple_of(r * H, H)
                        a = w_v[pl.ds(src, H // 2), :]
                        b = w_v[pl.ds(src + H // 2, H // 2), :]
                        dst = pl.ds(r, H // 2, stride=pitch)
                        wh_s[0, dst, :] = (a & U32(0xFFFF)) | (b << U32(16))
                        wh_s[1, dst, :] = (a >> U32(16)) | (b & U32(0xFFFF0000))
                    return carry
                lax.fori_loop(0, per_it // 8, body, 0)
                stream.pump(n)

        def head(h, rows):
            pitch = rows // 2 + 1
            return pltpu.bitcast(wh_s[h % 2, pl.ds(h // 2 * pitch, rows // 2), :], BF16)

        c_cp = pltpu.make_async_copy(c_hbm, c_v, sem_c)
        x_cp = pltpu.make_async_copy(x_hbm, x_v, sem_x)
        c_cp.start()
        x_cp.start()

        front = _Stream()
        front.add(wm_hbm, wm_v, sem_wm, 6 * M * 2)
        wm_end = len(front)
        front.add(wq_hbm, wq_v, sem_wq, D * 4)
        wq_end = len(front)
        front.add(wuk_hbm, wuk_v, sem_wuk, D * 4)
        wuk_end = len(front)
        for b in range(2):
            front.add(ckv_hbm, ckv_v, sems.at[b], Dc * 2, base=b * Sk, rows=Sk)
        front_total = len(front)

        def pump_until(stream, total, step):
            stream.pump(max(0, min(step, total) - (total - len(stream))))

        pump_until(front, front_total, LAG)
        c_cp.wait()
        c = c_v[...].astype(F32)
        sc = (c * jax.nn.sigmoid(c)).astype(BF16)
        x_cp.wait()
        x = x_v[...].astype(F32)
        xn = _layernorm(x)
        pump_until(front, front_total, wm_end + LAG)
        wait(wm_hbm, wm_v, sem_wm)
        mod = []
        for i in range(6):
            mod.append(_dot(sc, wm_v[:, i * M:(i + 1) * M]))
            front.pump(1)
        sa, ca, ga, sb, cb, gb = mod
        h = (xn * (1.0 + ca) + sa).astype(BF16)

        pump_until(front, front_total, wq_end + LAG)
        wait(wq_hbm, wq_v, sem_wq)
        split_heads(wq_v, M, front, [1] * 4)
        for i in range(H):
            q_s[i] = _dot(h, head(i, M))
            front.pump(i % 2)

        pump_until(front, front_total, wuk_end + LAG)
        wait(wuk_hbm, wuk_v, sem_wuk)
        split_heads(wuk_v, Dc, front, [1] * 4)
        for i in range(H):
            r = _dot_nt(q_s[i].astype(BF16), head(i, Dc)) * scale
            for t in range(n_ct):
                qa_s[t, pl.ds(i, B, stride=H), :] = r[:, t * LANES:(t + 1) * LANES]
            front.pump(i % 2)
        front.pump()

        def attend(b, stream, steps):
            r0 = b * H if isinstance(b, int) else pl.multiple_of(b * H, H)
            k0 = b * Sk if isinstance(b, int) else pl.multiple_of(b * Sk, Sk)
            steps = _spread(steps, 2 * n_kc)
            qb = jnp.concatenate(
                [qa_s[t, pl.ds(r0, H), :] for t in range(n_ct)], axis=1).astype(BF16)
            wait(ckv_hbm, ckv_v, sems.at[b], k0, Sk)
            mt = None
            for i in range(n_kc):
                s = _dot_nt(qb, ckv_v[pl.ds(k0 + i * KC, KC), :])
                s_s[:, i * KC:(i + 1) * KC] = s
                for t in range(KC // LANES):
                    st = s[:, t * LANES:(t + 1) * LANES]
                    mt = st if mt is None else jnp.maximum(mt, st)
                stream.pump(steps[i])
            m = jnp.max(mt, axis=1, keepdims=True)
            lt = None
            acc = None
            for i in range(n_kc):
                p = jnp.exp(s_s[:, i * KC:(i + 1) * KC] - m)
                for t in range(KC // LANES):
                    pt = p[:, t * LANES:(t + 1) * LANES]
                    lt = pt if lt is None else lt + pt
                d = _dot(p.astype(BF16), ckv_v[pl.ds(k0 + i * KC, KC), :])
                acc = d if acc is None else acc + d
                stream.pump(steps[n_kc + i])
            ctx = acc / jnp.sum(lt, axis=1, keepdims=True)
            for t in range(n_ct):
                ctx_s[t, pl.ds(r0, H), :] = ctx[:, t * LANES:(t + 1) * LANES]

        def attn_body(b, carry):
            stream = _Stream()
            stream.add(ckv_hbm, ckv_v, sems.at[b + 2], Dc * 2,
                       base=pl.multiple_of((b + 2) * Sk, Sk), rows=Sk)
            attend(b, stream, min(len(stream), ATTN_STEPS))
            stream.pump()
            return carry

        lax.fori_loop(0, B - 2, attn_body, 0)

        back = _Stream()
        back.add(wuv_hbm, wuv_v, sem_wuv, D * 4)
        wuv_end = len(back)
        back.add(wo_hbm, wo_v, sem_wo, M * 2)
        wo_end = len(back)
        back.add(w3_hbm, w3_v, sem_w3, F * 2)
        w3_end = len(back)
        for i, sem in enumerate(sem_w4):
            back.add(w4_hbm, w4_v, sem, M * 2, base=W4_CUTS[i], rows=W4_CUTS[i + 1] - W4_CUTS[i])
        back_total = len(back)

        attend(B - 2, back, TAIL_STEPS)
        pump_until(back, back_total, LAG)
        attend(B - 1, back, TAIL_STEPS)

        pump_until(back, back_total, wuv_end + LAG)
        wait(wuv_hbm, wuv_v, sem_wuv)
        split_heads(wuv_v, Dc, back, [1] * 4)
        for i in range(H):
            cx = jnp.concatenate(
                [ctx_s[t, pl.ds(i, B, stride=H), :] for t in range(n_ct)], axis=1).astype(BF16)
            cv_s[:, i * D:(i + 1) * D] = _dot(cx, head(i, Dc))
            back.pump(i % 2)

        pump_until(back, back_total, wo_end + LAG)
        wait(wo_hbm, wo_v, sem_wo)
        att = None
        for i in range(8):
            k = H * D // 8
            d = _dot(cv_s[:, i * k:(i + 1) * k].astype(BF16), wo_v[i * k:(i + 1) * k, :])
            att = d if att is None else att + d
            back.pump(1)
        x = x + ga * att
        h2 = _layernorm(x) * (1.0 + cb) + sb

        hn = _layernorm(h2).astype(BF16)
        back.pump()
        wait(w3_hbm, w3_v, sem_w3)
        g = jax.nn.gelu(_dot(hn, w3_v[...]), approximate=True).astype(BF16)
        y = h2
        for i, sem in enumerate(sem_w4):
            f0, f1 = W4_CUTS[i], W4_CUTS[i + 1]
            wait(w4_hbm, w4_v, sem, f0, f1 - f0)
            y = y + _dot(g[:, f0:f1], w4_v[f0:f1, :])
        o_ref[...] = (x + gb * y).astype(o_ref.dtype)

    return kernel


@jax.jit
def pallas_adaLN_cond__compressed_kv_cla__mixer_s_mlp__decode_kernel(
    A_x: jax.Array,
    A_c_kv: jax.Array,
    A_w_q: jax.Array,
    A_w_uk: jax.Array,
    A_w_uv: jax.Array,
    A_w_o: jax.Array,
    B_x: jax.Array,
    B_w1: jax.Array,
    B_w2: jax.Array,
    B_w3: jax.Array,
    B_w4: jax.Array,
    c: jax.Array,
    w_mod: jax.Array,
):
    B, Sq, M = A_x.shape
    _, Sk, Dc = A_c_kv.shape
    _, H, D = A_w_q.shape
    F = B_w3.shape[1]
    assert Sq == 1 and D == LANES

    ins = (
        A_x.reshape(B, M),
        A_c_kv.reshape(B * Sk, Dc),
        A_w_q.reshape(M * H, D),
        A_w_uk.reshape(Dc * H, D),
        A_w_uv.reshape(Dc * H, D),
        A_w_o.reshape(H * D, M),
        B_w3,
        B_w4,
        c,
        w_mod,
    )
    out = pl.pallas_call(
        _make_kernel(B, H, D, M, Dc, Sk, F),
        out_shape=jax.ShapeDtypeStruct((B, M), A_x.dtype),
        in_specs=[pl.BlockSpec(memory_space=pltpu.HBM)] * len(ins),
        out_specs=pl.BlockSpec(memory_space=pltpu.VMEM),
        scratch_shapes=[pltpu.VMEM((a.shape[0] // 2, D), U32) if i in (2, 3, 4) else pltpu.VMEM(a.shape, a.dtype) for i, a in enumerate(ins)] + [
            pltpu.VMEM((2, H // 2 * (max(M, Dc) // 2 + 1), D), U32),
            pltpu.VMEM((H, B, D), F32),
            pltpu.VMEM((Dc // LANES, B * H, LANES), F32),
            pltpu.VMEM((H, Sk), F32),
            pltpu.VMEM((Dc // LANES, B * H, LANES), F32),
            pltpu.VMEM((B, H * D), F32),
            pltpu.SemaphoreType.DMA((B + 8 + len(W4_CUTS) - 1,)),
        ],
        compiler_params=pltpu.CompilerParams(
            vmem_limit_bytes=100 * 1024 * 1024,
            disable_bounds_checks=NO_CHECKS, disable_semaphore_checks=NO_CHECKS),
    )(*ins)
    return out.reshape(B, Sq, M)
```

```python
import jax
import jax.numpy as jnp
from jax import lax
import jax.experimental.pallas as pl
import jax.experimental.pallas.tpu as pltpu

F32 = jnp.float32
BF16 = jnp.bfloat16
U32 = jnp.uint32
LANES = 128

REGIONS = 8
N_LO = 6
STEPS = 64
LAG = 32
ATTN_STEPS = 48
TAIL_STEPS = 32
W3_SPAN = (0.0, 0.8)
W4_SPAN = (0.6, 1.06)
W4_CUTS = (0, 384, 512)
NO_CHECKS = True


def _layernorm(x, eps=1e-5):
    m = jnp.mean(x, axis=-1, keepdims=True)
    d = x - m
    v = jnp.mean(d * d, axis=-1, keepdims=True)
    return d * lax.rsqrt(v + eps)


def _dot(a, b):
    return jnp.dot(a, b, preferred_element_type=F32)


def _dot_nt(a, b):
    return lax.dot_general(a, b, (((1,), (1,)), ((), ())), preferred_element_type=F32)


def _copy_steps(src, dst, sem_of, n_steps, n_lo, g0=0, groups=None, col_chunks=1):
    groups = src.shape[0] if groups is None else groups
    rows = src.shape[1] * col_chunks // n_steps
    cols = src.shape[2] // col_chunks
    steps = []
    for i in range(n_steps):
        r0 = i // col_chunks * rows
        rc = (pl.ds(r0, rows), pl.ds(i % col_chunks * cols, cols))
        parts = ((g0, n_lo, 1), (g0 + n_lo, groups - n_lo, 0))
        steps.append([(src, dst, sem_of(r0), (pl.ds(g, n), *rc), prio) for g, n, prio in parts if n])
    return steps


class _Stream:
    def __init__(self, spans):
        timed = [(t0 + (t1 - t0) * (i + 0.5) / len(steps), k, name, step)
                 for k, (name, steps, t0, t1) in enumerate(spans) for i, step in enumerate(steps)]
        timed.sort(key=lambda e: e[:2])
        self.steps = [e[3] for e in timed]
        self.end = {e[2]: i + 1 for i, e in enumerate(timed)}
        self.pos = 0

    def pump(self, n):
        for step in self.steps[self.pos:self.pos + n]:
            for src, dst, sem, idx, prio in step:
                pltpu.make_async_copy(src.at[idx], dst.at[idx], sem).start(priority=prio)
        self.pos = min(self.pos + n, len(self.steps))

    def pump_to(self, pos):
        self.pump(max(0, pos - self.pos))

    def pump_past(self, name):
        self.pump_to(self.end[name] + LAG)

    def flush(self):
        self.pump_to(len(self.steps))


def _spread(total, parts):
    return [total * (i + 1) // parts - total * i // parts for i in range(parts)]


def _make_kernel(B, H, D, M, Dc, Sk, F):
    scale = float(D) ** -0.5
    kc = Sk // REGIONS
    n_ct = Dc // LANES
    half = STEPS // 2
    w4_main = F // M * M

    def kernel(x_hbm, c_hbm, wm_hbm, wq_hbm, wuk_hbm, ckv_hbm, wuv_hbm, wo_hbm, w3_hbm, w4_hbm,
               o_ref,
               x_v, c_v, wm_v, wq_v, wuk_v, ckv_v, wuv_v, wo_v, w3_v, w4a_v, w4b_v,
               wh_s, q_s, qa_s, s_s, ctx_s, cv_s, sems):
        wq_hbm, wuk_hbm, wuv_hbm = (w.bitcast(U32) for w in (wq_hbm, wuk_hbm, wuv_hbm))
        w4a_hbm = w4_hbm.at[pl.ds(0, w4_main), :].reshape(w4a_v.shape)
        w4b_hbm = w4_hbm.at[pl.ds(w4_main, F - w4_main), :].reshape(w4b_v.shape)
        (sem_x, sem_c, sem_wm, sem_wq, sem_wuk, sem_wuv, sem_wo, sem_w3, sem_w4b, *sem_w4a) = (
            sems.at[B + i] for i in range(9 + len(W4_CUTS) - 1))

        def steps_of(src, dst, sem):
            return _copy_steps(src, dst, lambda r: sem, STEPS, N_LO)

        def ckv_steps(b):
            return _copy_steps(ckv_hbm, ckv_v, lambda r: sems.at[b], STEPS, N_LO,
                               g0=b * REGIONS, groups=REGIONS)

        def wait(src, dst, sem, idx=...):
            pltpu.make_async_copy(src.at[idx], dst.at[idx], sem).wait()

        def split_heads(w_v, stream):
            per_region = w_v.shape[1] // H
            pitch = REGIONS * per_region + 1
            for g in range(REGIONS):
                def body(i, carry):
                    for t in range(8):
                        r = i * 8 + t
                        src = pl.multiple_of(r * H, H)
                        a = w_v[g, pl.ds(src, H // 2), :]
                        b = w_v[g, pl.ds(src + H // 2, H // 2), :]
                        dst = pl.ds(g * per_region + r, H // 2, stride=pitch)
                        wh_s[0, dst, :] = (a & U32(0xFFFF)) | (b << U32(16))
                        wh_s[1, dst, :] = (a >> U32(16)) | (b & U32(0xFFFF0000))
                    return carry
                lax.fori_loop(0, per_region // 8, body, 0)
                stream.pump(1)

        def head(h, rows):
            pitch = rows // 2 + 1
            return pltpu.bitcast(wh_s[h % 2, pl.ds(h // 2 * pitch, rows // 2), :], BF16)

        c_cp = pltpu.make_async_copy(c_hbm, c_v, sem_c)
        x_cp = pltpu.make_async_copy(x_hbm, x_v, sem_x)
        c_cp.start()
        x_cp.start()

        front = _Stream([
            ("wm", _copy_steps(wm_hbm, wm_v, lambda r: sem_wm, 48, 3, col_chunks=3), -1.5, 0.5),
            ("wq", steps_of(wq_hbm, wq_v, sem_wq), -1.0, 1.0),
            ("wuk", steps_of(wuk_hbm, wuk_v, sem_wuk), 0.0, 2.0),
            ("k0", ckv_steps(0), 1.0, 3.0),
            ("k1", ckv_steps(1), 2.0, 4.0),
            ("k2", ckv_steps(2)[:half], 3.0, 4.0),
        ])

        front.pump(LAG)
        c_cp.wait()
        c = c_v[...].astype(F32)
        sc = (c * jax.nn.sigmoid(c)).astype(BF16)
        x_cp.wait()
        x = x_v[...].astype(F32)
        xn = _layernorm(x)
        front.pump_past("wm")
        wait(wm_hbm, wm_v, sem_wm)
        mod = []
        for i in range(6):
            w = wm_v[:, :, i * M:(i + 1) * M]
            mod.append(_dot(sc, w.reshape(-1, M)))
            front.pump(2)
        sa, ca, ga, sb, cb, gb = mod
        h = (xn * (1.0 + ca) + sa).astype(BF16)

        front.pump_past("wq")
        wait(wq_hbm, wq_v, sem_wq)
        split_heads(wq_v, front)
        for i in range(H):
            q_s[i] = _dot(h, head(i, M))
            front.pump(i % 2)

        front.pump_past("wuk")
        wait(wuk_hbm, wuk_v, sem_wuk)
        split_heads(wuk_v, front)
        for i in range(H):
            r = _dot_nt(q_s[i].astype(BF16), head(i, Dc)) * scale
            for t in range(n_ct):
                qa_s[t, pl.ds(i, B, stride=H), :] = r[:, t * LANES:(t + 1) * LANES]
            front.pump(i % 2)
        front.flush()

        def attend(b, stream, steps):
            r0 = b * H if isinstance(b, int) else pl.multiple_of(b * H, H)
            g0 = b * REGIONS
            steps = _spread(steps, 2 * REGIONS)
            qb = jnp.concatenate(
                [qa_s[t, pl.ds(r0, H), :] for t in range(n_ct)], axis=1).astype(BF16)
            wait(ckv_hbm, ckv_v, sems.at[b], pl.ds(g0, REGIONS))
            mt = None
            for i in range(REGIONS):
                s = _dot_nt(qb, ckv_v[g0 + i])
                s_s[:, i * kc:(i + 1) * kc] = s
                for t in range(kc // LANES):
                    st = s[:, t * LANES:(t + 1) * LANES]
                    mt = st if mt is None else jnp.maximum(mt, st)
                stream.pump(steps[i])
            m = jnp.max(mt, axis=1, keepdims=True)
            lt = None
            acc = None
            for i in range(REGIONS):
                p = jnp.exp(s_s[:, i * kc:(i + 1) * kc] - m)
                for t in range(kc // LANES):
                    pt = p[:, t * LANES:(t + 1) * LANES]
                    lt = pt if lt is None else lt + pt
                d = _dot(p.astype(BF16), ckv_v[g0 + i])
                acc = d if acc is None else acc + d
                stream.pump(steps[REGIONS + i])
            ctx = acc / jnp.sum(lt, axis=1, keepdims=True)
            for t in range(n_ct):
                ctx_s[t, pl.ds(r0, H), :] = ctx[:, t * LANES:(t + 1) * LANES]

        def attn_body(b, carry):
            stream = _Stream([("a", ckv_steps(b + 2)[half:], 0.0, 1.0),
                              ("b", ckv_steps(b + 3)[:half], 0.0, 1.0)])
            attend(b, stream, ATTN_STEPS)
            stream.flush()
            return carry

        lax.fori_loop(0, B - 3, attn_body, 0)

        def w4a_sem(r):
            return sem_w4a[sum(r >= cut for cut in W4_CUTS[1:])]

        w4_steps = [a + b for a, b in zip(_copy_steps(w4a_hbm, w4a_v, w4a_sem, 32, F // M),
                                          _copy_steps(w4b_hbm, w4b_v, lambda r: sem_w4b, 32, 0))]
        back = _Stream([
            ("k7", ckv_steps(B - 1)[half:], -2.0, -1.0),
            ("wuv", steps_of(wuv_hbm, wuv_v, sem_wuv), -2.0, 0.0),
            ("wo", steps_of(wo_hbm, wo_v, sem_wo)[:half], -1.0, 0.0),
            ("wo", steps_of(wo_hbm, wo_v, sem_wo)[half:], 0.0, 0.6),
            ("w3", _copy_steps(w3_hbm, w3_v, lambda r: sem_w3, 32, 3, col_chunks=2), *W3_SPAN),
            ("w4", w4_steps, *W4_SPAN),
        ])
        attend(B - 3, back, TAIL_STEPS)
        back.pump_to(LAG)
        attend(B - 2, back, TAIL_STEPS)
        back.pump_past("k7")
        attend(B - 1, back, TAIL_STEPS)

        back.pump_past("wuv")
        wait(wuv_hbm, wuv_v, sem_wuv)
        split_heads(wuv_v, back)
        for i in range(H):
            cx = jnp.concatenate(
                [ctx_s[t, pl.ds(i, B, stride=H), :] for t in range(n_ct)], axis=1).astype(BF16)
            cv_s[:, i * D:(i + 1) * D] = _dot(cx, head(i, Dc))
            back.pump(i % 2)

        back.pump_past("wo")
        wait(wo_hbm, wo_v, sem_wo)
        att = None
        k = H * D // REGIONS
        for i in range(REGIONS):
            d = _dot(cv_s[:, i * k:(i + 1) * k].astype(BF16), wo_v[i])
            att = d if att is None else att + d
            back.pump(1)
        x = x + ga * att
        h2 = _layernorm(x) * (1.0 + cb) + sb

        hn = _layernorm(h2).astype(BF16)
        back.flush()
        wait(w3_hbm, w3_v, sem_w3)
        g = jax.nn.gelu(_dot(hn, w3_v[...].reshape(M, F)), approximate=True).astype(BF16)
        wait(w4b_hbm, w4b_v, sem_w4b)
        y = h2 + _dot(g[:, w4_main:], w4b_v[0])
        for i, sem in enumerate(sem_w4a):
            f0, f1 = W4_CUTS[i], W4_CUTS[i + 1]
            wait(w4a_hbm, w4a_v, sem, (slice(None), pl.ds(f0, f1 - f0)))
            for j in range(F // M):
                y = y + _dot(g[:, j * M + f0:j * M + f1], w4a_v[j, f0:f1, :])
        o_ref[...] = (x + gb * y).astype(o_ref.dtype)

    return kernel


@jax.jit
def pallas_adaLN_cond__compressed_kv_cla__mixer_s_mlp__decode_kernel(
    A_x: jax.Array,
    A_c_kv: jax.Array,
    A_w_q: jax.Array,
    A_w_uk: jax.Array,
    A_w_uv: jax.Array,
    A_w_o: jax.Array,
    B_x: jax.Array,
    B_w1: jax.Array,
    B_w2: jax.Array,
    B_w3: jax.Array,
    B_w4: jax.Array,
    c: jax.Array,
    w_mod: jax.Array,
):
    B, Sq, M = A_x.shape
    _, Sk, Dc = A_c_kv.shape
    _, H, D = A_w_q.shape
    F = B_w3.shape[1]
    assert Sq == 1 and D == LANES

    ins = (
        A_x.reshape(B, M),
        c,
        w_mod.reshape(4, -1, 6 * M),
        A_w_q.reshape(REGIONS, -1, D),
        A_w_uk.reshape(REGIONS, -1, D),
        A_c_kv.reshape(B * REGIONS, Sk // REGIONS, Dc),
        A_w_uv.reshape(REGIONS, -1, D),
        A_w_o.reshape(REGIONS, -1, M),
        B_w3.reshape(4, -1, F),
        B_w4,
    )

    def like(a):
        return pltpu.VMEM(a.shape, a.dtype)

    def words(a):
        return pltpu.VMEM((a.shape[0], a.shape[1] // 2, a.shape[2]), U32)

    out = pl.pallas_call(
        _make_kernel(B, H, D, M, Dc, Sk, F),
        out_shape=jax.ShapeDtypeStruct((B, M), A_x.dtype),
        in_specs=[pl.BlockSpec(memory_space=pltpu.HBM)] * len(ins),
        out_specs=pl.BlockSpec(memory_space=pltpu.VMEM),
        scratch_shapes=[
            like(ins[0]), like(ins[1]), like(ins[2]), words(ins[3]), words(ins[4]), like(ins[5]),
            words(ins[6]), like(ins[7]), like(ins[8]),
            pltpu.VMEM((F // M, M, M), B_w4.dtype),
            pltpu.VMEM((1, F % M, M), B_w4.dtype),
            pltpu.VMEM((2, H // 2 * (max(M, Dc) // 2 + 1), D), U32),
            pltpu.VMEM((H, B, D), F32),
            pltpu.VMEM((Dc // LANES, B * H, LANES), F32),
            pltpu.VMEM((H, Sk), F32),
            pltpu.VMEM((Dc // LANES, B * H, LANES), F32),
            pltpu.VMEM((B, H * D), F32),
            pltpu.SemaphoreType.DMA((B + 9 + len(W4_CUTS) - 1,)),
        ],
        compiler_params=pltpu.CompilerParams(
            vmem_limit_bytes=100 * 1024 * 1024,
            disable_bounds_checks=NO_CHECKS, disable_semaphore_checks=NO_CHECKS),
    )(*ins)
    return out.reshape(B, Sq, M)
```

```python
import jax
import jax.numpy as jnp
from jax import lax
import jax.experimental.pallas as pl
import jax.experimental.pallas.tpu as pltpu

F32 = jnp.float32
BF16 = jnp.bfloat16
U32 = jnp.uint32
LANES = 128

REGIONS = 8
SPLIT = ((7, 1), (1, 0))
STEPS = 64
LAG = 32
ATTN_STEPS = 48
TAIL_STEPS = 32
WO_SPAN = (0.0, 0.6)
W3_SPAN = (0.0, 0.8)
W4_SPAN = (0.6, 1.06)
W4_CUTS = (0, 384, 512)
NO_CHECKS = True
FIRST = 4
WM_CUT = (96, ((3, 1), (1, 0)), 6)
W3_CUT = (32, ((3, 1), (1, 0)), 2)
WM_SPAN = (-1.5, 0.5)
W4_STEPS = 32


def _layernorm(x, eps=1e-5):
    m = jnp.mean(x, axis=-1, keepdims=True)
    d = x - m
    v = jnp.mean(d * d, axis=-1, keepdims=True)
    return d * lax.rsqrt(v + eps)


def _dot(a, b):
    return jnp.dot(a, b, preferred_element_type=F32)


def _dot_nt(a, b):
    return lax.dot_general(a, b, (((1,), (1,)), ((), ())), preferred_element_type=F32)


def _copy_steps(src, dst, sem_of, n_steps, split, col_chunks=1, g0=0):
    rows = src.shape[1] * col_chunks // n_steps
    cols = src.shape[2] // col_chunks
    steps = []
    for i in range(n_steps):
        r0 = i // col_chunks * rows
        rc = (pl.ds(r0, rows), pl.ds(i % col_chunks * cols, cols))
        step, g = [], 0
        for n, prio in split:
            step.append((src, dst, sem_of(r0), (pl.ds(g0 + g, n), *rc), prio))
            g += n
        steps.append(step)
    return steps


class _Stream:
    def __init__(self, spans):
        timed = [(t0 + (t1 - t0) * (i + 0.5) / len(steps), k, name, step)
                 for k, (name, steps, t0, t1) in enumerate(spans) for i, step in enumerate(steps)]
        timed.sort(key=lambda e: e[:2])
        self.steps = [e[3] for e in timed]
        self.end = {e[2]: i + 1 for i, e in enumerate(timed)}
        self.pos = 0

    def pump(self, n):
        for step in self.steps[self.pos:self.pos + n]:
            for src, dst, sem, idx, prio in step:
                pltpu.make_async_copy(src.at[idx], dst.at[idx], sem).start(priority=prio)
        self.pos = min(self.pos + n, len(self.steps))

    def pump_to(self, pos):
        self.pump(max(0, pos - self.pos))

    def pump_past(self, name):
        self.pump_to(self.end[name] + LAG)

    def flush(self):
        self.pump_to(len(self.steps))


def _spread(total, parts):
    return [total * (i + 1) // parts - total * i // parts for i in range(parts)]


def _make_kernel(B, H, D, M, Dc, Sk, F):
    scale = float(D) ** -0.5
    kc = Sk // REGIONS
    n_ct = Dc // LANES
    half = STEPS // 2
    w4_main = F // M * M

    def kernel(x_hbm, c_hbm, wm_hbm, wq_hbm, wuk_hbm, ckv_hbm, wuv_hbm, wo_hbm, w3_hbm, w4_hbm,
               o_ref,
               x_v, c_v, wm_v, wq_v, wuk_v, ckv_v, wuv_v, wo_v, w3_v, w4a_v, w4b_v,
               wh_s, q_s, qa_s, s_s, ctx_s, cv_s, sems):
        wq_hbm, wuk_hbm, wuv_hbm = (w.bitcast(U32) for w in (wq_hbm, wuk_hbm, wuv_hbm))
        w4a_hbm = w4_hbm.at[pl.ds(0, w4_main), :].reshape(w4a_v.shape)
        w4b_hbm = w4_hbm.at[pl.ds(w4_main, F - w4_main), :].reshape(w4b_v.shape)
        (sem_x, sem_c, sem_wm, sem_wq, sem_wuk, sem_wuv, sem_wo, sem_w3, sem_w4b, *sem_w4a) = (
            sems.at[B + i] for i in range(9 + len(W4_CUTS) - 1))

        def steps_of(src, dst, sem):
            return _copy_steps(src, dst, lambda r: sem, STEPS, SPLIT)

        def ckv_steps(b):
            return _copy_steps(ckv_hbm, ckv_v, lambda r: sems.at[b], STEPS, SPLIT, g0=b * REGIONS)

        def wait(src, dst, sem, idx=...):
            pltpu.make_async_copy(src.at[idx], dst.at[idx], sem).wait()

        def split_heads(w_v, stream):
            per_region = w_v.shape[1] // H
            pitch = REGIONS * per_region + 1
            for g in range(REGIONS):
                def body(i, carry):
                    for t in range(8):
                        r = i * 8 + t
                        src = pl.multiple_of(r * H, H)
                        a = w_v[g, pl.ds(src, H // 2), :]
                        b = w_v[g, pl.ds(src + H // 2, H // 2), :]
                        dst = pl.ds(g * per_region + r, H // 2, stride=pitch)
                        wh_s[0, dst, :] = (a & U32(0xFFFF)) | (b << U32(16))
                        wh_s[1, dst, :] = (a >> U32(16)) | (b & U32(0xFFFF0000))
                    return carry
                lax.fori_loop(0, per_region // 8, body, 0)
                stream.pump(1)

        def head(h, rows):
            pitch = rows // 2 + 1
            return pltpu.bitcast(wh_s[h % 2, pl.ds(h // 2 * pitch, rows // 2), :], BF16)

        c_cp = pltpu.make_async_copy(c_hbm, c_v, sem_c)
        x_cp = pltpu.make_async_copy(x_hbm, x_v, sem_x)

        front = _Stream([
            ("wm", _copy_steps(wm_hbm, wm_v, lambda r: sem_wm, *WM_CUT), *WM_SPAN),
            ("wq", steps_of(wq_hbm, wq_v, sem_wq), -1.0, 1.0),
            ("wuk", steps_of(wuk_hbm, wuk_v, sem_wuk), 0.0, 2.0),
            ("k0", ckv_steps(0), 1.0, 3.0),
            ("k1", ckv_steps(1), 2.0, 4.0),
            ("k2", ckv_steps(2)[:half], 3.0, 4.0),
        ])

        front.pump(FIRST)
        c_cp.start()
        x_cp.start()
        front.pump_to(LAG)
        c_cp.wait()
        c = c_v[...].astype(F32)
        sc = (c * jax.nn.sigmoid(c)).astype(BF16)
        x_cp.wait()
        x = x_v[...].astype(F32)
        xn = _layernorm(x)
        front.pump_past("wm")
        wait(wm_hbm, wm_v, sem_wm)
        mod = []
        for i in range(6):
            w = wm_v[:, :, i * M:(i + 1) * M]
            mod.append(_dot(sc, w.reshape(-1, M)))
            front.pump(2)
        sa, ca, ga, sb, cb, gb = mod
        h = (xn * (1.0 + ca) + sa).astype(BF16)

        front.pump_past("wq")
        wait(wq_hbm, wq_v, sem_wq)
        split_heads(wq_v, front)
        for i in range(H):
            q_s[i] = _dot(h, head(i, M))
            front.pump(i % 2)

        front.pump_past("wuk")
        wait(wuk_hbm, wuk_v, sem_wuk)
        split_heads(wuk_v, front)
        for i in range(H):
            r = _dot_nt(q_s[i].astype(BF16), head(i, Dc)) * scale
            for t in range(n_ct):
                qa_s[t, pl.ds(i, B, stride=H), :] = r[:, t * LANES:(t + 1) * LANES]
            front.pump(i % 2)
        front.flush()

        def attend(b, stream, steps):
            r0 = b * H if isinstance(b, int) else pl.multiple_of(b * H, H)
            g0 = b * REGIONS
            steps = _spread(steps, 2 * REGIONS)
            qb = jnp.concatenate(
                [qa_s[t, pl.ds(r0, H), :] for t in range(n_ct)], axis=1).astype(BF16)
            wait(ckv_hbm, ckv_v, sems.at[b], pl.ds(g0, REGIONS))
            mt = None
            for i in range(REGIONS):
                s = _dot_nt(qb, ckv_v[g0 + i])
                s_s[:, i * kc:(i + 1) * kc] = s
                for t in range(kc // LANES):
                    st = s[:, t * LANES:(t + 1) * LANES]
                    mt = st if mt is None else jnp.maximum(mt, st)
                stream.pump(steps[i])
            m = jnp.max(mt, axis=1, keepdims=True)
            lt = None
            acc = None
            for i in range(REGIONS):
                p = jnp.exp(s_s[:, i * kc:(i + 1) * kc] - m)
                for t in range(kc // LANES):
                    pt = p[:, t * LANES:(t + 1) * LANES]
                    lt = pt if lt is None else lt + pt
                d = _dot(p.astype(BF16), ckv_v[g0 + i])
                acc = d if acc is None else acc + d
                stream.pump(steps[REGIONS + i])
            ctx = acc / jnp.sum(lt, axis=1, keepdims=True)
            for t in range(n_ct):
                ctx_s[t, pl.ds(r0, H), :] = ctx[:, t * LANES:(t + 1) * LANES]

        def attn_body(b, carry):
            stream = _Stream([("a", ckv_steps(b + 2)[half:], 0.0, 1.0),
                              ("b", ckv_steps(b + 3)[:half], 0.0, 1.0)])
            attend(b, stream, ATTN_STEPS)
            stream.flush()
            return carry

        lax.fori_loop(0, B - 3, attn_body, 0)

        def w4a_sem(r):
            return sem_w4a[sum(r >= cut for cut in W4_CUTS[1:])]

        w4a_steps = _copy_steps(w4a_hbm, w4a_v, w4a_sem, W4_STEPS, ((F // M, 1),))
        w4b_steps = _copy_steps(w4b_hbm, w4b_v, lambda r: sem_w4b, 32, ((1, 0),))
        k = W4_STEPS // 32
        w4_steps = [sum(w4a_steps[i * k:(i + 1) * k], []) + w4b_steps[i] for i in range(32)]
        back = _Stream([
            ("k7", ckv_steps(B - 1)[half:], -2.0, -1.0),
            ("wuv", steps_of(wuv_hbm, wuv_v, sem_wuv), -2.0, 0.0),
            ("wo", steps_of(wo_hbm, wo_v, sem_wo)[:half], -1.0, 0.0),
            ("wo", steps_of(wo_hbm, wo_v, sem_wo)[half:], *WO_SPAN),
            ("w3", _copy_steps(w3_hbm, w3_v, lambda r: sem_w3, *W3_CUT), *W3_SPAN),
            ("w4", w4_steps, *W4_SPAN),
        ])
        attend(B - 3, back, TAIL_STEPS)
        back.pump_to(LAG)
        attend(B - 2, back, TAIL_STEPS)
        back.pump_past("k7")
        attend(B - 1, back, TAIL_STEPS)

        back.pump_past("wuv")
        wait(wuv_hbm, wuv_v, sem_wuv)
        split_heads(wuv_v, back)
        for i in range(H):
            cx = jnp.concatenate(
                [ctx_s[t, pl.ds(i, B, stride=H), :] for t in range(n_ct)], axis=1).astype(BF16)
            cv_s[:, i * D:(i + 1) * D] = _dot(cx, head(i, Dc))
            back.pump(i % 2)

        back.pump_past("wo")
        wait(wo_hbm, wo_v, sem_wo)
        att = None
        k = H * D // REGIONS
        for i in range(REGIONS):
            d = _dot(cv_s[:, i * k:(i + 1) * k].astype(BF16), wo_v[i])
            att = d if att is None else att + d
            back.pump(1)
        x = x + ga * att
        h2 = _layernorm(x) * (1.0 + cb) + sb

        hn = _layernorm(h2).astype(BF16)
        back.flush()
        wait(w3_hbm, w3_v, sem_w3)
        g = jax.nn.gelu(_dot(hn, w3_v[...].reshape(M, F)), approximate=True).astype(BF16)
        wait(w4b_hbm, w4b_v, sem_w4b)
        y = h2 + _dot(g[:, w4_main:], w4b_v[0])
        for i, sem in enumerate(sem_w4a):
            f0, f1 = W4_CUTS[i], W4_CUTS[i + 1]
            wait(w4a_hbm, w4a_v, sem, (slice(None), pl.ds(f0, f1 - f0)))
            for j in range(F // M):
                y = y + _dot(g[:, j * M + f0:j * M + f1], w4a_v[j, f0:f1, :])
        o_ref[...] = (x + gb * y).astype(o_ref.dtype)

    return kernel


@jax.jit
def pallas_adaLN_cond__compressed_kv_cla__mixer_s_mlp__decode_kernel(
    A_x: jax.Array,
    A_c_kv: jax.Array,
    A_w_q: jax.Array,
    A_w_uk: jax.Array,
    A_w_uv: jax.Array,
    A_w_o: jax.Array,
    B_x: jax.Array,
    B_w1: jax.Array,
    B_w2: jax.Array,
    B_w3: jax.Array,
    B_w4: jax.Array,
    c: jax.Array,
    w_mod: jax.Array,
):
    B, Sq, M = A_x.shape
    _, Sk, Dc = A_c_kv.shape
    _, H, D = A_w_q.shape
    F = B_w3.shape[1]
    assert Sq == 1 and D == LANES

    ins = (
        A_x.reshape(B, M),
        c,
        w_mod.reshape(sum(n for n, _ in WM_CUT[1]), -1, 6 * M),
        A_w_q.reshape(REGIONS, -1, D),
        A_w_uk.reshape(REGIONS, -1, D),
        A_c_kv.reshape(B * REGIONS, Sk // REGIONS, Dc),
        A_w_uv.reshape(REGIONS, -1, D),
        A_w_o.reshape(REGIONS, -1, M),
        B_w3.reshape(sum(n for n, _ in W3_CUT[1]), -1, F),
        B_w4,
    )

    def like(a):
        return pltpu.VMEM(a.shape, a.dtype)

    def words(a):
        return pltpu.VMEM((a.shape[0], a.shape[1] // 2, a.shape[2]), U32)

    out = pl.pallas_call(
        _make_kernel(B, H, D, M, Dc, Sk, F),
        out_shape=jax.ShapeDtypeStruct((B, M), A_x.dtype),
        in_specs=[pl.BlockSpec(memory_space=pltpu.HBM)] * len(ins),
        out_specs=pl.BlockSpec(memory_space=pltpu.VMEM),
        scratch_shapes=[
            like(ins[0]), like(ins[1]), like(ins[2]), words(ins[3]), words(ins[4]), like(ins[5]),
            words(ins[6]), like(ins[7]), like(ins[8]),
            pltpu.VMEM((F // M, M, M), B_w4.dtype),
            pltpu.VMEM((1, F % M, M), B_w4.dtype),
            pltpu.VMEM((2, H // 2 * (max(M, Dc) // 2 + 1), D), U32),
            pltpu.VMEM((H, B, D), F32),
            pltpu.VMEM((Dc // LANES, B * H, LANES), F32),
            pltpu.VMEM((H, Sk), F32),
            pltpu.VMEM((Dc // LANES, B * H, LANES), F32),
            pltpu.VMEM((B, H * D), F32),
            pltpu.SemaphoreType.DMA((B + 9 + len(W4_CUTS) - 1,)),
        ],
        compiler_params=pltpu.CompilerParams(
            vmem_limit_bytes=100 * 1024 * 1024,
            disable_bounds_checks=NO_CHECKS, disable_semaphore_checks=NO_CHECKS),
    )(*ins)
    return out.reshape(B, Sq, M)
```

```python
import jax
import jax.numpy as jnp
from jax import lax
import jax.experimental.pallas as pl
import jax.experimental.pallas.tpu as pltpu

F32 = jnp.float32
BF16 = jnp.bfloat16
U32 = jnp.uint32
LANES = 128

LO, HI = 1, 0
REGIONS = 8
STEPS = 64
SPLIT = ((7, LO), (1, HI))
SMALL_SPLIT = ((3, LO), (1, HI))
LAG = 32
ATTN_STEPS = 48
LATE_ATTN_STEPS = 32
W4_CUTS = (0, 384, 512)


def _layernorm(x, eps=1e-5):
    d = x - jnp.mean(x, axis=-1, keepdims=True)
    return d * lax.rsqrt(jnp.mean(d * d, axis=-1, keepdims=True) + eps)


def _dot(a, b):
    return jnp.dot(a, b, preferred_element_type=F32)


def _dot_nt(a, b):
    return lax.dot_general(a, b, (((1,), (1,)), ((), ())), preferred_element_type=F32)


def _copy_steps(src, dst, sem_of, n_steps, split, col_chunks=1, g0=0):
    rows = src.shape[1] * col_chunks // n_steps
    cols = src.shape[2] // col_chunks
    assert rows * n_steps == src.shape[1] * col_chunks and cols * col_chunks == src.shape[2]
    steps = []
    for i in range(n_steps):
        r0 = i // col_chunks * rows
        slab = (pl.ds(r0, rows), pl.ds(i % col_chunks * cols, cols))
        step, g = [], 0
        for n, priority in split:
            step.append((src, dst, sem_of(r0), (pl.ds(g0 + g, n), *slab), priority))
            g += n
        steps.append(step)
    return steps


class _Stream:
    def __init__(self, spans):
        timed = [(t0 + (t1 - t0) * (i + 0.5) / len(steps), k, name, step)
                 for k, (name, steps, t0, t1) in enumerate(spans) for i, step in enumerate(steps)]
        timed.sort(key=lambda e: e[:2])
        self.steps = [e[3] for e in timed]
        self.end = {e[2]: i + 1 for i, e in enumerate(timed)}
        self.pos = 0

    def pump(self, n):
        for step in self.steps[self.pos:self.pos + n]:
            for src, dst, sem, idx, priority in step:
                pltpu.make_async_copy(src.at[idx], dst.at[idx], sem).start(priority=priority)
        self.pos = min(self.pos + n, len(self.steps))

    def pump_to(self, pos):
        self.pump(max(0, pos - self.pos))

    def pump_past(self, name):
        self.pump_to(self.end[name] + LAG)

    def flush(self):
        self.pump_to(len(self.steps))


def _make_kernel(B, H, D, M, Dc, Sk, F):
    scale = float(D) ** -0.5
    kc = Sk // REGIONS
    n_ct = Dc // LANES
    half = STEPS // 2
    n_f = F // M

    def kernel(x_hbm, c_hbm, wm_hbm, wq_hbm, wuk_hbm, ckv_hbm, wuv_hbm, wo_hbm, w3_hbm, w4_hbm,
               o_ref,
               x_v, c_v, wm_v, wq_v, wuk_v, ckv_v, wuv_v, wo_v, w3_v, w4a_v, w4b_v,
               wh_s, q_s, qa_s, s_s, ctx_s, cv_s, sems):
        wq_hbm, wuk_hbm, wuv_hbm = (w.bitcast(U32) for w in (wq_hbm, wuk_hbm, wuv_hbm))
        w4a_hbm = w4_hbm.at[pl.ds(0, n_f * M), :].reshape(w4a_v.shape)
        w4b_hbm = w4_hbm.at[pl.ds(n_f * M, F - n_f * M), :].reshape(w4b_v.shape)
        (sem_x, sem_c, sem_wm, sem_wq, sem_wuk, sem_wuv, sem_wo, sem_w3, sem_w4b, *sem_w4a) = (
            sems.at[i] for i in range(B, sems.shape[0]))

        def steps_of(src, dst, sem):
            return _copy_steps(src, dst, lambda r: sem, STEPS, SPLIT)

        def ckv_steps(b):
            return _copy_steps(ckv_hbm, ckv_v, lambda r: sems.at[b], STEPS, SPLIT, g0=b * REGIONS)

        def wait(src, dst, sem, idx=...):
            pltpu.make_async_copy(src.at[idx], dst.at[idx], sem).wait()

        def split_heads(w_v, stream):
            per_region = w_v.shape[1] // H
            pitch = REGIONS * per_region + 1
            for g in range(REGIONS):
                def body(i, carry, g=g):
                    for t in range(8):
                        r = i * 8 + t
                        src = pl.multiple_of(r * H, H)
                        even = w_v[g, pl.ds(src, H // 2), :]
                        odd = w_v[g, pl.ds(src + H // 2, H // 2), :]
                        dst = pl.ds(g * per_region + r, H // 2, stride=pitch)
                        wh_s[0, dst, :] = (even & U32(0xFFFF)) | (odd << U32(16))
                        wh_s[1, dst, :] = (even >> U32(16)) | (odd & U32(0xFFFF0000))
                    return carry
                lax.fori_loop(0, per_region // 8, body, 0)
                stream.pump(1)

        def head(h, rows):
            pitch = rows // 2 + 1
            return pltpu.bitcast(wh_s[h % 2, pl.ds(h // 2 * pitch, rows // 2), :], BF16)

        front = _Stream([
            ("wm", _copy_steps(wm_hbm, wm_v, lambda r: sem_wm, 96, SMALL_SPLIT, 6), -1.5, 0.5),
            ("wq", steps_of(wq_hbm, wq_v, sem_wq), -1.0, 1.0),
            ("wuk", steps_of(wuk_hbm, wuk_v, sem_wuk), 0.0, 2.0),
            ("k0", ckv_steps(0), 1.0, 3.0),
            ("k1", ckv_steps(1), 2.0, 4.0),
            ("k2", ckv_steps(2)[:half], 3.0, 4.0),
        ])

        c_cp = pltpu.make_async_copy(c_hbm, c_v, sem_c)
        x_cp = pltpu.make_async_copy(x_hbm, x_v, sem_x)
        front.pump(4)
        c_cp.start()
        x_cp.start()
        front.pump_to(LAG)
        c_cp.wait()
        c = c_v[...].astype(F32)
        sc = (c * jax.nn.sigmoid(c)).astype(BF16)
        x_cp.wait()
        x = x_v[...].astype(F32)
        xn = _layernorm(x)
        front.pump_past("wm")
        wait(wm_hbm, wm_v, sem_wm)
        mod = []
        for i in range(6):
            mod.append(_dot(sc, wm_v[:, :, i * M:(i + 1) * M].reshape(-1, M)))
            front.pump(2)
        sa, ca, ga, sb, cb, gb = mod
        h = (xn * (1.0 + ca) + sa).astype(BF16)

        front.pump_past("wq")
        wait(wq_hbm, wq_v, sem_wq)
        split_heads(wq_v, front)
        for i in range(H):
            q_s[i] = _dot(h, head(i, M))
            front.pump(i % 2)

        front.pump_past("wuk")
        wait(wuk_hbm, wuk_v, sem_wuk)
        split_heads(wuk_v, front)
        for i in range(H):
            r = _dot_nt(q_s[i].astype(BF16), head(i, Dc)) * scale
            for t in range(n_ct):
                qa_s[t, pl.ds(i, B, stride=H), :] = r[:, t * LANES:(t + 1) * LANES]
            front.pump(i % 2)
        front.flush()

        def attend(b, stream, steps):
            r0 = b * H if isinstance(b, int) else pl.multiple_of(b * H, H)
            g0 = b * REGIONS
            per_chunk = steps // (2 * REGIONS)
            qb = jnp.concatenate(
                [qa_s[t, pl.ds(r0, H), :] for t in range(n_ct)], axis=1).astype(BF16)
            wait(ckv_hbm, ckv_v, sems.at[b], pl.ds(g0, REGIONS))
            mt = None
            for i in range(REGIONS):
                s = _dot_nt(qb, ckv_v[g0 + i])
                s_s[:, i * kc:(i + 1) * kc] = s
                for t in range(kc // LANES):
                    st = s[:, t * LANES:(t + 1) * LANES]
                    mt = st if mt is None else jnp.maximum(mt, st)
                stream.pump(per_chunk)
            m = jnp.max(mt, axis=1, keepdims=True)
            lt = None
            acc = None
            for i in range(REGIONS):
                p = jnp.exp(s_s[:, i * kc:(i + 1) * kc] - m)
                for t in range(kc // LANES):
                    pt = p[:, t * LANES:(t + 1) * LANES]
                    lt = pt if lt is None else lt + pt
                d = _dot(p.astype(BF16), ckv_v[g0 + i])
                acc = d if acc is None else acc + d
                stream.pump(per_chunk)
            ctx = acc / jnp.sum(lt, axis=1, keepdims=True)
            for t in range(n_ct):
                ctx_s[t, pl.ds(r0, H), :] = ctx[:, t * LANES:(t + 1) * LANES]

        def attn_body(b, carry):
            stream = _Stream([("a", ckv_steps(b + 2)[half:], 0.0, 1.0),
                              ("b", ckv_steps(b + 3)[:half], 0.0, 1.0)])
            attend(b, stream, ATTN_STEPS)
            stream.flush()
            return carry

        lax.fori_loop(0, B - 3, attn_body, 0)

        def w4a_sem(r):
            return sem_w4a[sum(r >= cut for cut in W4_CUTS[1:])]

        w4_steps = [a + b for a, b in zip(
            _copy_steps(w4a_hbm, w4a_v, w4a_sem, 32, ((n_f, LO),)),
            _copy_steps(w4b_hbm, w4b_v, lambda r: sem_w4b, 32, ((1, HI),)))]
        wo_steps = steps_of(wo_hbm, wo_v, sem_wo)
        back = _Stream([
            ("k7", ckv_steps(B - 1)[half:], -2.0, -1.0),
            ("wuv", steps_of(wuv_hbm, wuv_v, sem_wuv), -2.0, 0.0),
            ("wo", wo_steps[:half], -1.0, 0.0),
            ("wo", wo_steps[half:], 0.0, 0.6),
            ("w3", _copy_steps(w3_hbm, w3_v, lambda r: sem_w3, 32, SMALL_SPLIT, 2), 0.0, 0.8),
            ("w4", w4_steps, 0.6, 1.06),
        ])
        attend(B - 3, back, LATE_ATTN_STEPS)
        back.pump_to(LAG)
        attend(B - 2, back, LATE_ATTN_STEPS)
        back.pump_past("k7")
        attend(B - 1, back, LATE_ATTN_STEPS)

        back.pump_past("wuv")
        wait(wuv_hbm, wuv_v, sem_wuv)
        split_heads(wuv_v, back)
        for i in range(H):
            cx = jnp.concatenate(
                [ctx_s[t, pl.ds(i, B, stride=H), :] for t in range(n_ct)], axis=1).astype(BF16)
            cv_s[:, i * D:(i + 1) * D] = _dot(cx, head(i, Dc))
            back.pump(i % 2)

        back.pump_past("wo")
        wait(wo_hbm, wo_v, sem_wo)
        att = None
        k = H * D // REGIONS
        for i in range(REGIONS):
            d = _dot(cv_s[:, i * k:(i + 1) * k].astype(BF16), wo_v[i])
            att = d if att is None else att + d
            back.pump(1)
        x = x + ga * att
        h2 = _layernorm(x) * (1.0 + cb) + sb

        hn = _layernorm(h2).astype(BF16)
        back.flush()
        wait(w3_hbm, w3_v, sem_w3)
        g = jax.nn.gelu(_dot(hn, w3_v[...].reshape(M, F)), approximate=True).astype(BF16)
        wait(w4b_hbm, w4b_v, sem_w4b)
        y = h2 + _dot(g[:, n_f * M:], w4b_v[0])
        for i, sem in enumerate(sem_w4a):
            f0, f1 = W4_CUTS[i], W4_CUTS[i + 1]
            wait(w4a_hbm, w4a_v, sem, (slice(None), pl.ds(f0, f1 - f0)))
            for j in range(n_f):
                y = y + _dot(g[:, j * M + f0:j * M + f1], w4a_v[j, f0:f1, :])
        o_ref[...] = (x + gb * y).astype(o_ref.dtype)

    return kernel


@jax.jit
def pallas_adaLN_cond__compressed_kv_cla__mixer_s_mlp__decode_kernel(
    A_x: jax.Array,
    A_c_kv: jax.Array,
    A_w_q: jax.Array,
    A_w_uk: jax.Array,
    A_w_uv: jax.Array,
    A_w_o: jax.Array,
    B_x: jax.Array,
    B_w1: jax.Array,
    B_w2: jax.Array,
    B_w3: jax.Array,
    B_w4: jax.Array,
    c: jax.Array,
    w_mod: jax.Array,
):
    B, Sq, M = A_x.shape
    _, Sk, Dc = A_c_kv.shape
    _, H, D = A_w_q.shape
    F = B_w3.shape[1]
    assert Sq == 1 and D == LANES and M == W4_CUTS[-1]
    small_regions = sum(n for n, _ in SMALL_SPLIT)

    ins = (
        A_x.reshape(B, M),
        c,
        w_mod.reshape(small_regions, -1, 6 * M),
        A_w_q.reshape(REGIONS, -1, D),
        A_w_uk.reshape(REGIONS, -1, D),
        A_c_kv.reshape(B * REGIONS, Sk // REGIONS, Dc),
        A_w_uv.reshape(REGIONS, -1, D),
        A_w_o.reshape(REGIONS, -1, M),
        B_w3.reshape(small_regions, -1, F),
        B_w4,
    )

    def like(a):
        return pltpu.VMEM(a.shape, a.dtype)

    def words(a):
        return pltpu.VMEM((a.shape[0], a.shape[1] // 2, a.shape[2]), U32)

    out = pl.pallas_call(
        _make_kernel(B, H, D, M, Dc, Sk, F),
        out_shape=jax.ShapeDtypeStruct((B, M), A_x.dtype),
        in_specs=[pl.BlockSpec(memory_space=pltpu.HBM)] * len(ins),
        out_specs=pl.BlockSpec(memory_space=pltpu.VMEM),
        scratch_shapes=[
            like(ins[0]), like(ins[1]), like(ins[2]), words(ins[3]), words(ins[4]), like(ins[5]),
            words(ins[6]), like(ins[7]), like(ins[8]),
            pltpu.VMEM((F // M, M, M), B_w4.dtype),
            pltpu.VMEM((1, F % M, M), B_w4.dtype),
            pltpu.VMEM((2, (H // 2 + 1) * (max(M, Dc) // 2 + 1), D), U32),
            pltpu.VMEM((H, B, D), F32),
            pltpu.VMEM((Dc // LANES, (B + 1) * H, LANES), F32),
            pltpu.VMEM((H, Sk), F32),
            pltpu.VMEM((Dc // LANES, (B + 1) * H, LANES), F32),
            pltpu.VMEM((B, H * D), F32),
            pltpu.SemaphoreType.DMA((B + 9 + len(W4_CUTS) - 1,)),
        ],
        compiler_params=pltpu.CompilerParams(
            vmem_limit_bytes=100 * 1024 * 1024,
            disable_bounds_checks=True,
            disable_semaphore_checks=True,
        ),
    )(*ins)
    return out.reshape(B, Sq, M)
```

```python
import jax
import jax.numpy as jnp
from jax import lax
import jax.experimental.pallas as pl
import jax.experimental.pallas.tpu as pltpu

F32 = jnp.float32
BF16 = jnp.bfloat16
U32 = jnp.uint32
LANES = 128

LO, HI = 1, 0
REGIONS = 8
STEPS = 64
SPLIT = ((7, LO), (1, HI))
SMALL_SPLIT = ((3, LO), (1, HI))
LAG = 32
ATTN_STEPS = 48
LATE_ATTN_STEPS = 32
W4_CUTS = (0, 384, 512)


def _layernorm(x, eps=1e-5):
    d = x - jnp.mean(x, axis=-1, keepdims=True)
    return d * lax.rsqrt(jnp.mean(d * d, axis=-1, keepdims=True) + eps)


def _dot(a, b):
    return jnp.dot(a, b, preferred_element_type=F32)


def _dot_nt(a, b):
    return lax.dot_general(a, b, (((1,), (1,)), ((), ())), preferred_element_type=F32)


def _copy_steps(src, dst, sem_of, n_steps, split, col_chunks=1, g0=0):
    rows = src.shape[1] * col_chunks // n_steps
    cols = src.shape[2] // col_chunks
    assert rows * n_steps == src.shape[1] * col_chunks and cols * col_chunks == src.shape[2]
    steps = []
    for i in range(n_steps):
        r0 = i // col_chunks * rows
        slab = (pl.ds(r0, rows), pl.ds(i % col_chunks * cols, cols))
        step, g = [], 0
        for n, priority in split:
            step.append((src, dst, sem_of(r0), (pl.ds(g0 + g, n), *slab), priority))
            g += n
        steps.append(step)
    return steps


class _Stream:
    def __init__(self, spans):
        timed = [(t0 + (t1 - t0) * (i + 0.5) / len(steps), k, name, step)
                 for k, (name, steps, t0, t1) in enumerate(spans) for i, step in enumerate(steps)]
        timed.sort(key=lambda e: e[:2])
        self.steps = [e[3] for e in timed]
        self.end = {e[2]: i + 1 for i, e in enumerate(timed)}
        self.pos = 0

    def pump(self, n):
        for step in self.steps[self.pos:self.pos + n]:
            for src, dst, sem, idx, priority in step:
                pltpu.make_async_copy(src.at[idx], dst.at[idx], sem).start(priority=priority)
        self.pos = min(self.pos + n, len(self.steps))

    def pump_to(self, pos):
        self.pump(max(0, pos - self.pos))

    def pump_past(self, name):
        self.pump_to(self.end[name] + LAG)

    def flush(self):
        self.pump_to(len(self.steps))


def _make_kernel(B, H, D, M, Dc, Sk, F):
    scale = float(D) ** -0.5
    kc = Sk // REGIONS
    n_ct = Dc // LANES
    half = STEPS // 2
    n_f = F // M

    def kernel(x_hbm, c_hbm, wm_hbm, wq_hbm, wuk_hbm, ckv_hbm, wuv_hbm, wo_hbm, w3_hbm, w4_hbm,
               o_ref,
               x_v, c_v, wm_v, wq_v, wuk_v, ckv_v, wuv_v, wo_v, w3_v, w4a_v, w4b_v,
               wh_s, q_s, qa_s, s_s, ctx_s, cv_s, sems):
        w4a_hbm = w4_hbm.at[pl.ds(0, n_f * M), :].reshape(w4a_v.shape)
        w4b_hbm = w4_hbm.at[pl.ds(n_f * M, F - n_f * M), :].reshape(w4b_v.shape)
        (sem_x, sem_c, sem_wm, sem_wq, sem_wuk, sem_wuv, sem_wo, sem_w3, sem_w4b, *sem_w4a) = (
            sems.at[i] for i in range(B, sems.shape[0]))

        def steps_of(src, dst, sem):
            return _copy_steps(src, dst, lambda r: sem, STEPS, SPLIT)

        def ckv_steps(b):
            return _copy_steps(ckv_hbm, ckv_v, lambda r: sems.at[b], STEPS, SPLIT, g0=b * REGIONS)

        def wait(src, dst, sem, idx=...):
            pltpu.make_async_copy(src.at[idx], dst.at[idx], sem).wait()

        def split_heads(w_v, stream):
            per_region = w_v.shape[1] // (2 * H)
            pitch = REGIONS * per_region + 1
            for g in range(REGIONS):
                def body(i, carry, g=g):
                    for t in range(8):
                        r = i * 8 + t
                        src = pl.multiple_of(r * 2 * H, 2 * H)
                        even = pltpu.bitcast(w_v[g, pl.ds(src, H), :], U32)
                        odd = pltpu.bitcast(w_v[g, pl.ds(src + H, H), :], U32)
                        dst = pl.ds(g * per_region + r, H // 2, stride=pitch)
                        wh_s[0, dst, :] = (even & U32(0xFFFF)) | (odd << U32(16))
                        wh_s[1, dst, :] = (even >> U32(16)) | (odd & U32(0xFFFF0000))
                    return carry
                lax.fori_loop(0, per_region // 8, body, 0)
                stream.pump(1)

        def head(h, rows):
            pitch = rows // 2 + 1
            return pltpu.bitcast(wh_s[h % 2, pl.ds(h // 2 * pitch, rows // 2), :], BF16)

        front = _Stream([
            ("wm", _copy_steps(wm_hbm, wm_v, lambda r: sem_wm, 96, SMALL_SPLIT, 6), -1.5, 0.5),
            ("wq", steps_of(wq_hbm, wq_v, sem_wq), -1.0, 1.0),
            ("wuk", steps_of(wuk_hbm, wuk_v, sem_wuk), 0.0, 2.0),
            ("k0", ckv_steps(0), 1.0, 3.0),
            ("k1", ckv_steps(1), 2.0, 4.0),
            ("k2", ckv_steps(2)[:half], 3.0, 4.0),
        ])

        c_cp = pltpu.make_async_copy(c_hbm, c_v, sem_c)
        x_cp = pltpu.make_async_copy(x_hbm, x_v, sem_x)
        front.pump(4)
        c_cp.start()
        x_cp.start()
        front.pump_to(LAG)
        c_cp.wait()
        c = c_v[...].astype(F32)
        sc = (c * jax.nn.sigmoid(c)).astype(BF16)
        x_cp.wait()
        x = x_v[...].astype(F32)
        xn = _layernorm(x)
        front.pump_past("wm")
        wait(wm_hbm, wm_v, sem_wm)
        mod = []
        for i in range(6):
            mod.append(_dot(sc, wm_v[:, :, i * M:(i + 1) * M].reshape(-1, M)))
            front.pump(2)
        sa, ca, ga, sb, cb, gb = mod
        h = (xn * (1.0 + ca) + sa).astype(BF16)

        front.pump_past("wq")
        wait(wq_hbm, wq_v, sem_wq)
        split_heads(wq_v, front)
        for i in range(H):
            q_s[i] = _dot(h, head(i, M))
            front.pump(i % 2)

        front.pump_past("wuk")
        wait(wuk_hbm, wuk_v, sem_wuk)
        split_heads(wuk_v, front)
        for i in range(H):
            r = _dot_nt(q_s[i].astype(BF16), head(i, Dc)) * scale
            for t in range(n_ct):
                qa_s[t, pl.ds(i, B, stride=H), :] = r[:, t * LANES:(t + 1) * LANES]
            front.pump(i % 2)
        front.flush()

        def attend(b, stream, steps):
            r0 = b * H if isinstance(b, int) else pl.multiple_of(b * H, H)
            g0 = b * REGIONS
            per_chunk = steps // (2 * REGIONS)
            qb = jnp.concatenate(
                [qa_s[t, pl.ds(r0, H), :] for t in range(n_ct)], axis=1).astype(BF16)
            wait(ckv_hbm, ckv_v, sems.at[b], pl.ds(g0, REGIONS))
            mt = None
            for i in range(REGIONS):
                s = _dot_nt(qb, ckv_v[g0 + i])
                s_s[:, i * kc:(i + 1) * kc] = s
                for t in range(kc // LANES):
                    st = s[:, t * LANES:(t + 1) * LANES]
                    mt = st if mt is None else jnp.maximum(mt, st)
                stream.pump(per_chunk)
            m = jnp.max(mt, axis=1, keepdims=True)
            lt = None
            acc = None
            for i in range(REGIONS):
                p = jnp.exp(s_s[:, i * kc:(i + 1) * kc] - m)
                for t in range(kc // LANES):
                    pt = p[:, t * LANES:(t + 1) * LANES]
                    lt = pt if lt is None else lt + pt
                d = _dot(p.astype(BF16), ckv_v[g0 + i])
                acc = d if acc is None else acc + d
                stream.pump(per_chunk)
            ctx = acc / jnp.sum(lt, axis=1, keepdims=True)
            for t in range(n_ct):
                ctx_s[t, pl.ds(r0, H), :] = ctx[:, t * LANES:(t + 1) * LANES]

        def attn_body(b, carry):
            stream = _Stream([("a", ckv_steps(b + 2)[half:], 0.0, 1.0),
                              ("b", ckv_steps(b + 3)[:half], 0.0, 1.0)])
            attend(b, stream, ATTN_STEPS)
            stream.flush()
            return carry

        lax.fori_loop(0, B - 3, attn_body, 0)

        def w4a_sem(r):
            return sem_w4a[sum(r >= cut for cut in W4_CUTS[1:])]

        w4_steps = [a + b for a, b in zip(
            _copy_steps(w4a_hbm, w4a_v, w4a_sem, 32, ((n_f, LO),)),
            _copy_steps(w4b_hbm, w4b_v, lambda r: sem_w4b, 32, ((1, HI),)))]
        wo_steps = steps_of(wo_hbm, wo_v, sem_wo)
        back = _Stream([
            ("k7", ckv_steps(B - 1)[half:], -2.0, -1.0),
            ("wuv", steps_of(wuv_hbm, wuv_v, sem_wuv), -2.0, 0.0),
            ("wo", wo_steps[:half], -1.0, 0.0),
            ("wo", wo_steps[half:], 0.0, 0.6),
            ("w3", _copy_steps(w3_hbm, w3_v, lambda r: sem_w3, 32, SMALL_SPLIT, 2), 0.0, 0.8),
            ("w4", w4_steps, 0.6, 1.06),
        ])
        attend(B - 3, back, LATE_ATTN_STEPS)
        back.pump_to(LAG)
        attend(B - 2, back, LATE_ATTN_STEPS)
        back.pump_past("k7")
        attend(B - 1, back, LATE_ATTN_STEPS)

        back.pump_past("wuv")
        wait(wuv_hbm, wuv_v, sem_wuv)
        split_heads(wuv_v, back)
        for i in range(H):
            cx = jnp.concatenate(
                [ctx_s[t, pl.ds(i, B, stride=H), :] for t in range(n_ct)], axis=1).astype(BF16)
            cv_s[:, i * D:(i + 1) * D] = _dot(cx, head(i, Dc))
            back.pump(i % 2)

        back.pump_past("wo")
        wait(wo_hbm, wo_v, sem_wo)
        att = None
        k = H * D // REGIONS
        for i in range(REGIONS):
            d = _dot(cv_s[:, i * k:(i + 1) * k].astype(BF16), wo_v[i])
            att = d if att is None else att + d
            back.pump(1)
        x = x + ga * att
        h2 = _layernorm(x) * (1.0 + cb) + sb

        hn = _layernorm(h2).astype(BF16)
        back.flush()
        wait(w3_hbm, w3_v, sem_w3)
        g = jax.nn.gelu(_dot(hn, w3_v[...].reshape(M, F)), approximate=True).astype(BF16)
        wait(w4b_hbm, w4b_v, sem_w4b)
        y = h2 + _dot(g[:, n_f * M:], w4b_v[0])
        for i, sem in enumerate(sem_w4a):
            f0, f1 = W4_CUTS[i], W4_CUTS[i + 1]
            wait(w4a_hbm, w4a_v, sem, (slice(None), pl.ds(f0, f1 - f0)))
            for j in range(n_f):
                y = y + _dot(g[:, j * M + f0:j * M + f1], w4a_v[j, f0:f1, :])
        o_ref[...] = (x + gb * y).astype(o_ref.dtype)

    return kernel


@jax.jit
def pallas_adaLN_cond__compressed_kv_cla__mixer_s_mlp__decode_kernel(
    A_x: jax.Array,
    A_c_kv: jax.Array,
    A_w_q: jax.Array,
    A_w_uk: jax.Array,
    A_w_uv: jax.Array,
    A_w_o: jax.Array,
    B_x: jax.Array,
    B_w1: jax.Array,
    B_w2: jax.Array,
    B_w3: jax.Array,
    B_w4: jax.Array,
    c: jax.Array,
    w_mod: jax.Array,
):
    B, Sq, M = A_x.shape
    _, Sk, Dc = A_c_kv.shape
    _, H, D = A_w_q.shape
    F = B_w3.shape[1]
    assert Sq == 1 and D == LANES and M == W4_CUTS[-1]
    small_regions = sum(n for n, _ in SMALL_SPLIT)

    ins = (
        A_x.reshape(B, M),
        c,
        w_mod.reshape(small_regions, -1, 6 * M),
        A_w_q.reshape(REGIONS, -1, D),
        A_w_uk.reshape(REGIONS, -1, D),
        A_c_kv.reshape(B * REGIONS, Sk // REGIONS, Dc),
        A_w_uv.reshape(REGIONS, -1, D),
        A_w_o.reshape(REGIONS, -1, M),
        B_w3.reshape(small_regions, -1, F),
        B_w4,
    )
    out = pl.pallas_call(
        _make_kernel(B, H, D, M, Dc, Sk, F),
        out_shape=jax.ShapeDtypeStruct((B, M), A_x.dtype),
        in_specs=[pl.BlockSpec(memory_space=pltpu.HBM)] * len(ins),
        out_specs=pl.BlockSpec(memory_space=pltpu.VMEM),
        scratch_shapes=[
            *(pltpu.VMEM(a.shape, a.dtype) for a in ins[:-1]),
            pltpu.VMEM((F // M, M, M), B_w4.dtype),
            pltpu.VMEM((1, F % M, M), B_w4.dtype),
            pltpu.VMEM((2, (H // 2 + 1) * (max(M, Dc) // 2 + 1), D), U32),
            pltpu.VMEM((H, B, D), F32),
            pltpu.VMEM((Dc // LANES, (B + 1) * H, LANES), F32),
            pltpu.VMEM((H, Sk), F32),
            pltpu.VMEM((Dc // LANES, (B + 1) * H, LANES), F32),
            pltpu.VMEM((B, H * D), F32),
            pltpu.SemaphoreType.DMA((B + 9 + len(W4_CUTS) - 1,)),
        ],
        compiler_params=pltpu.CompilerParams(
            vmem_limit_bytes=100 * 1024 * 1024,
            disable_bounds_checks=True,
            disable_semaphore_checks=True,
        ),
    )(*ins)
    return out.reshape(B, Sq, M)
```

```python
import jax
import jax.numpy as jnp
from jax import lax
import jax.experimental.pallas as pl
import jax.experimental.pallas.tpu as pltpu

F32 = jnp.float32
BF16 = jnp.bfloat16
U32 = jnp.uint32
LANES = 128

LO, HI = 1, 0
REGIONS = 8
STEPS = 64
SPLIT = ((7, LO), (1, HI))
SMALL_SPLIT = ((3, LO), (1, HI))
LAG = 32
ATTN_STEPS = 48
LATE_ATTN_STEPS = 32
W4_ROWS = 48


def _layernorm(x, eps=1e-5):
    d = x - jnp.mean(x, axis=-1, keepdims=True)
    return d * lax.rsqrt(jnp.mean(d * d, axis=-1, keepdims=True) + eps)


def _dot(a, b):
    return jnp.dot(a, b, preferred_element_type=F32)


def _dot_nt(a, b):
    return lax.dot_general(a, b, (((1,), (1,)), ((), ())), preferred_element_type=F32)


def _copy_steps(src, dst, sem_of, n_steps, split, col_chunks=1, g0=0):
    rows = src.shape[1] * col_chunks // n_steps
    cols = src.shape[2] // col_chunks
    assert rows * n_steps == src.shape[1] * col_chunks and cols * col_chunks == src.shape[2]
    steps = []
    for i in range(n_steps):
        r0 = i // col_chunks * rows
        slab = (pl.ds(r0, rows), pl.ds(i % col_chunks * cols, cols))
        step, g = [], 0
        for n, priority in split:
            step.append((src, dst, sem_of(r0), (pl.ds(g0 + g, n), *slab), priority))
            g += n
        steps.append(step)
    return steps


class _Stream:
    def __init__(self, spans):
        timed = [(t0 + (t1 - t0) * (i + 0.5) / len(steps), k, name, step)
                 for k, (name, steps, t0, t1) in enumerate(spans) for i, step in enumerate(steps)]
        timed.sort(key=lambda e: e[:2])
        self.steps = [e[3] for e in timed]
        self.end = {e[2]: i + 1 for i, e in enumerate(timed)}
        self.pos = 0

    def pump(self, n):
        for step in self.steps[self.pos:self.pos + n]:
            for src, dst, sem, idx, priority in step:
                pltpu.make_async_copy(src.at[idx], dst.at[idx], sem).start(priority=priority)
        self.pos = min(self.pos + n, len(self.steps))

    def pump_to(self, pos):
        self.pump(max(0, pos - self.pos))

    def pump_past(self, name):
        self.pump_to(self.end[name] + LAG)

    def flush(self):
        self.pump_to(len(self.steps))


def _make_kernel(B, H, D, M, Dc, Sk, F):
    scale = float(D) ** -0.5
    kc = Sk // REGIONS
    n_ct = Dc // LANES
    half = STEPS // 2
    n_f = F // M
    w4_parts = ([(n_f * M, F)] + [(j * M, (j + 1) * M - LANES) for j in range(n_f)]
                + [((j + 1) * M - LANES, (j + 1) * M) for j in range(n_f)])

    def kernel(x_hbm, c_hbm, wm_hbm, wq_hbm, wuk_hbm, ckv_hbm, wuv_hbm, wo_hbm, w3_hbm, w4_hbm,
               o_ref,
               x_v, c_v, wm_v, wq_v, wuk_v, ckv_v, wuv_v, wo_v, w3_v, w4_v,
               wh_s, q_s, qa_s, s_s, ctx_s, cv_s, sems):
        (sem_x, sem_c, sem_wm, sem_wq, sem_wuk, sem_wuv, sem_wo, sem_w3, *sem_w4) = (
            sems.at[i] for i in range(B, sems.shape[0]))

        def steps_of(src, dst, sem):
            return _copy_steps(src, dst, lambda r: sem, STEPS, SPLIT)

        def ckv_steps(b):
            return _copy_steps(ckv_hbm, ckv_v, lambda r: sems.at[b], STEPS, SPLIT, g0=b * REGIONS)

        def wait(src, dst, sem, idx=...):
            pltpu.make_async_copy(src.at[idx], dst.at[idx], sem).wait()

        def split_heads(w_v, stream):
            per_region = w_v.shape[1] // (2 * H)
            pitch = REGIONS * per_region + 1
            for g in range(REGIONS):
                def body(i, carry, g=g):
                    for t in range(8):
                        r = i * 8 + t
                        src = pl.multiple_of(r * 2 * H, 2 * H)
                        even = pltpu.bitcast(w_v[g, pl.ds(src, H), :], U32)
                        odd = pltpu.bitcast(w_v[g, pl.ds(src + H, H), :], U32)
                        dst = pl.ds(g * per_region + r, H // 2, stride=pitch)
                        wh_s[0, dst, :] = (even & U32(0xFFFF)) | (odd << U32(16))
                        wh_s[1, dst, :] = (even >> U32(16)) | (odd & U32(0xFFFF0000))
                    return carry
                lax.fori_loop(0, per_region // 8, body, 0)
                stream.pump(1)

        def head(h, rows):
            pitch = rows // 2 + 1
            return pltpu.bitcast(wh_s[h % 2, pl.ds(h // 2 * pitch, rows // 2), :], BF16)

        front = _Stream([
            ("wm", _copy_steps(wm_hbm, wm_v, lambda r: sem_wm, 96, SMALL_SPLIT, 6), -1.5, 0.5),
            ("wq", steps_of(wq_hbm, wq_v, sem_wq), -1.0, 1.0),
            ("wuk", steps_of(wuk_hbm, wuk_v, sem_wuk), 0.0, 2.0),
            ("k0", ckv_steps(0), 1.0, 3.0),
            ("k1", ckv_steps(1), 2.0, 4.0),
            ("k2", ckv_steps(2)[:half], 3.0, 4.0),
        ])

        c_cp = pltpu.make_async_copy(c_hbm, c_v, sem_c)
        x_cp = pltpu.make_async_copy(x_hbm, x_v, sem_x)
        front.pump(4)
        c_cp.start()
        x_cp.start()
        front.pump_to(LAG)
        c_cp.wait()
        c = c_v[...].astype(F32)
        sc = (c * jax.nn.sigmoid(c)).astype(BF16)
        x_cp.wait()
        x = x_v[...].astype(F32)
        xn = _layernorm(x)
        front.pump_past("wm")
        wait(wm_hbm, wm_v, sem_wm)
        mod = []
        for i in range(6):
            mod.append(_dot(sc, wm_v[:, :, i * M:(i + 1) * M].reshape(-1, M)))
            front.pump(2)
        sa, ca, ga, sb, cb, gb = mod
        h = (xn * (1.0 + ca) + sa).astype(BF16)

        front.pump_past("wq")
        wait(wq_hbm, wq_v, sem_wq)
        split_heads(wq_v, front)
        for i in range(H):
            q_s[i] = _dot(h, head(i, M))
            front.pump(i % 2)

        front.pump_past("wuk")
        wait(wuk_hbm, wuk_v, sem_wuk)
        split_heads(wuk_v, front)
        for i in range(H):
            r = _dot_nt(q_s[i].astype(BF16), head(i, Dc)) * scale
            for t in range(n_ct):
                qa_s[t, pl.ds(i, B, stride=H), :] = r[:, t * LANES:(t + 1) * LANES]
            front.pump(i % 2)
        front.flush()

        def attend(b, stream, steps):
            r0 = b * H if isinstance(b, int) else pl.multiple_of(b * H, H)
            g0 = b * REGIONS
            per_chunk = steps // (2 * REGIONS)
            qb = jnp.concatenate(
                [qa_s[t, pl.ds(r0, H), :] for t in range(n_ct)], axis=1).astype(BF16)
            wait(ckv_hbm, ckv_v, sems.at[b], pl.ds(g0, REGIONS))
            mt = None
            for i in range(REGIONS):
                s = _dot_nt(qb, ckv_v[g0 + i])
                s_s[:, i * kc:(i + 1) * kc] = s
                for t in range(kc // LANES):
                    st = s[:, t * LANES:(t + 1) * LANES]
                    mt = st if mt is None else jnp.maximum(mt, st)
                stream.pump(per_chunk)
            m = jnp.max(mt, axis=1, keepdims=True)
            lt = None
            acc = None
            for i in range(REGIONS):
                p = jnp.exp(s_s[:, i * kc:(i + 1) * kc] - m)
                for t in range(kc // LANES):
                    pt = p[:, t * LANES:(t + 1) * LANES]
                    lt = pt if lt is None else lt + pt
                d = _dot(p.astype(BF16), ckv_v[g0 + i])
                acc = d if acc is None else acc + d
                stream.pump(per_chunk)
            ctx = acc / jnp.sum(lt, axis=1, keepdims=True)
            for t in range(n_ct):
                ctx_s[t, pl.ds(r0, H), :] = ctx[:, t * LANES:(t + 1) * LANES]

        def attn_body(b, carry):
            stream = _Stream([("a", ckv_steps(b + 2)[half:], 0.0, 1.0),
                              ("b", ckv_steps(b + 3)[:half], 0.0, 1.0)])
            attend(b, stream, ATTN_STEPS)
            stream.flush()
            return carry

        lax.fori_loop(0, B - 3, attn_body, 0)

        def w4_copies(part, rows, priority):
            r0, r1 = w4_parts[part]
            return [(w4_hbm, w4_v, sem_w4[part], pl.ds(r, min(rows, r1 - r)), priority)
                    for r in range(r0, r1, rows)]

        w4_lo = [cp for first in (1, 1 + n_f)
                 for cps in zip(*(w4_copies(first + j, W4_ROWS, LO) for j in range(n_f)))
                 for cp in cps]
        w4_hi = w4_copies(0, 8, HI)
        w4_steps = [[cp] + w4_hi[i:i + 1] for i, cp in enumerate(w4_lo)]
        assert len(w4_lo) >= len(w4_hi)
        wo_steps = steps_of(wo_hbm, wo_v, sem_wo)
        back = _Stream([
            ("k7", ckv_steps(B - 1)[half:], -2.0, -1.0),
            ("wuv", steps_of(wuv_hbm, wuv_v, sem_wuv), -2.0, 0.0),
            ("wo", wo_steps[:half], -1.0, 0.0),
            ("wo", wo_steps[half:], 0.0, 0.6),
            ("w3", _copy_steps(w3_hbm, w3_v, lambda r: sem_w3, 32, SMALL_SPLIT, 2), 0.0, 0.8),
            ("w4", w4_steps, 0.6, 1.06),
        ])
        attend(B - 3, back, LATE_ATTN_STEPS)
        back.pump_to(LAG)
        attend(B - 2, back, LATE_ATTN_STEPS)
        back.pump_past("k7")
        attend(B - 1, back, LATE_ATTN_STEPS)

        back.pump_past("wuv")
        wait(wuv_hbm, wuv_v, sem_wuv)
        split_heads(wuv_v, back)
        for i in range(H):
            cx = jnp.concatenate(
                [ctx_s[t, pl.ds(i, B, stride=H), :] for t in range(n_ct)], axis=1).astype(BF16)
            cv_s[:, i * D:(i + 1) * D] = _dot(cx, head(i, Dc))
            back.pump(i % 2)

        back.pump_past("wo")
        wait(wo_hbm, wo_v, sem_wo)
        att = None
        k = H * D // REGIONS
        for i in range(REGIONS):
            d = _dot(cv_s[:, i * k:(i + 1) * k].astype(BF16), wo_v[i])
            att = d if att is None else att + d
            back.pump(1)
        x = x + ga * att
        h2 = _layernorm(x) * (1.0 + cb) + sb

        hn = _layernorm(h2).astype(BF16)
        back.flush()
        wait(w3_hbm, w3_v, sem_w3)
        g = jax.nn.gelu(_dot(hn, w3_v[...].reshape(M, F)), approximate=True).astype(BF16)
        y = h2
        for parts in (range(0, 1), range(1, 1 + n_f), range(1 + n_f, 1 + 2 * n_f)):
            for i in parts:
                r0, r1 = w4_parts[i]
                wait(w4_hbm, w4_v, sem_w4[i], pl.ds(r0, r1 - r0))
            for i in parts:
                r0, r1 = w4_parts[i]
                y = y + _dot(g[:, r0:r1], w4_v[r0:r1, :])
        o_ref[...] = (x + gb * y).astype(o_ref.dtype)

    return kernel


@jax.jit
def pallas_adaLN_cond__compressed_kv_cla__mixer_s_mlp__decode_kernel(
    A_x: jax.Array,
    A_c_kv: jax.Array,
    A_w_q: jax.Array,
    A_w_uk: jax.Array,
    A_w_uv: jax.Array,
    A_w_o: jax.Array,
    B_x: jax.Array,
    B_w1: jax.Array,
    B_w2: jax.Array,
    B_w3: jax.Array,
    B_w4: jax.Array,
    c: jax.Array,
    w_mod: jax.Array,
):
    B, Sq, M = A_x.shape
    _, Sk, Dc = A_c_kv.shape
    _, H, D = A_w_q.shape
    F = B_w3.shape[1]
    assert Sq == 1 and D == LANES
    small_regions = sum(n for n, _ in SMALL_SPLIT)

    ins = (
        A_x.reshape(B, M),
        c,
        w_mod.reshape(small_regions, -1, 6 * M),
        A_w_q.reshape(REGIONS, -1, D),
        A_w_uk.reshape(REGIONS, -1, D),
        A_c_kv.reshape(B * REGIONS, Sk // REGIONS, Dc),
        A_w_uv.reshape(REGIONS, -1, D),
        A_w_o.reshape(REGIONS, -1, M),
        B_w3.reshape(small_regions, -1, F),
        B_w4,
    )
    out = pl.pallas_call(
        _make_kernel(B, H, D, M, Dc, Sk, F),
        out_shape=jax.ShapeDtypeStruct((B, M), A_x.dtype),
        in_specs=[pl.BlockSpec(memory_space=pltpu.HBM)] * len(ins),
        out_specs=pl.BlockSpec(memory_space=pltpu.VMEM),
        scratch_shapes=[
            *(pltpu.VMEM(a.shape, a.dtype) for a in ins),
            pltpu.VMEM((2, (H // 2 + 1) * (max(M, Dc) // 2 + 1), D), U32),
            pltpu.VMEM((H, B, D), F32),
            pltpu.VMEM((Dc // LANES, (B + 1) * H, LANES), F32),
            pltpu.VMEM((H, Sk), F32),
            pltpu.VMEM((Dc // LANES, (B + 1) * H, LANES), F32),
            pltpu.VMEM((B, H * D), F32),
            pltpu.SemaphoreType.DMA((B + 9 + 2 * (F // M),)),
        ],
        compiler_params=pltpu.CompilerParams(
            vmem_limit_bytes=100 * 1024 * 1024,
            disable_bounds_checks=True,
            disable_semaphore_checks=True,
        ),
    )(*ins)
    return out.reshape(B, Sq, M)
```

```python
import jax
import jax.numpy as jnp
from jax import lax
import jax.experimental.pallas as pl
import jax.experimental.pallas.tpu as pltpu

F32 = jnp.float32
BF16 = jnp.bfloat16
U32 = jnp.uint32
LANES = 128

LO, HI = 1, 0
REGIONS = 8
STEPS = 64
SPLIT = ((7, LO), (1, HI))
SMALL_SPLIT = ((3, LO), (1, HI))
LAG = 32
ATTN_STEPS = 48
LATE_ATTN_STEPS = 32
W4_CUTS = (0, 1024, 1280, 1664, 1792)


def _layernorm(x, eps=1e-5):
    d = x - jnp.mean(x, axis=-1, keepdims=True)
    return d * lax.rsqrt(jnp.mean(d * d, axis=-1, keepdims=True) + eps)


def _dot(a, b):
    return jnp.dot(a, b, preferred_element_type=F32)


def _dot_nt(a, b):
    return lax.dot_general(a, b, (((1,), (1,)), ((), ())), preferred_element_type=F32)


def _copy_steps(src, dst, sem_of, n_steps, split, col_chunks=1, g0=0):
    rows = src.shape[1] * col_chunks // n_steps
    cols = src.shape[2] // col_chunks
    assert rows * n_steps == src.shape[1] * col_chunks and cols * col_chunks == src.shape[2]
    steps = []
    for i in range(n_steps):
        r0 = i // col_chunks * rows
        slab = (pl.ds(r0, rows), pl.ds(i % col_chunks * cols, cols))
        step, g = [], 0
        for n, priority in split:
            step.append((src, dst, sem_of(r0), (pl.ds(g0 + g, n), *slab), priority))
            g += n
        steps.append(step)
    return steps


class _Stream:
    def __init__(self, spans):
        timed = [(t0 + (t1 - t0) * (i + 0.5) / len(steps), k, name, step)
                 for k, (name, steps, t0, t1) in enumerate(spans) for i, step in enumerate(steps)]
        timed.sort(key=lambda e: e[:2])
        self.steps = [e[3] for e in timed]
        self.end = {e[2]: i + 1 for i, e in enumerate(timed)}
        self.pos = 0

    def pump(self, n):
        for step in self.steps[self.pos:self.pos + n]:
            for src, dst, sem, idx, priority in step:
                pltpu.make_async_copy(src.at[idx], dst.at[idx], sem).start(priority=priority)
        self.pos = min(self.pos + n, len(self.steps))

    def pump_to(self, pos):
        self.pump(max(0, pos - self.pos))

    def pump_past(self, name):
        self.pump_to(self.end[name] + LAG)

    def flush(self):
        self.pump_to(len(self.steps))


def _make_kernel(B, H, D, M, Dc, Sk, F):
    scale = float(D) ** -0.5
    kc = Sk // REGIONS
    n_ct = Dc // LANES
    half = STEPS // 2

    def kernel(x_hbm, c_hbm, wm_hbm, wq_hbm, wuk_hbm, ckv_hbm, wuv_hbm, wo_hbm, w3_hbm, w4_hbm,
               o_ref,
               x_v, c_v, wm_v, wq_v, wuk_v, ckv_v, wuv_v, wo_v, w3_v, w4_v,
               wh_s, q_s, qa_s, s_s, ctx_s, cv_s, sems):
        (sem_x, sem_c, sem_wm, sem_wq, sem_wuk, sem_wuv, sem_wo, sem_w3, *sem_w4) = (
            sems.at[i] for i in range(B, sems.shape[0]))

        def steps_of(src, dst, sem):
            return _copy_steps(src, dst, lambda r: sem, STEPS, SPLIT)

        def ckv_steps(b):
            return _copy_steps(ckv_hbm, ckv_v, lambda r: sems.at[b], STEPS, SPLIT, g0=b * REGIONS)

        def wait(src, dst, sem, idx=...):
            pltpu.make_async_copy(src.at[idx], dst.at[idx], sem).wait()

        def split_heads(w_v, stream):
            per_region = w_v.shape[1] // (2 * H)
            pitch = REGIONS * per_region + 1
            for g in range(REGIONS):
                def body(i, carry, g=g):
                    for t in range(8):
                        r = i * 8 + t
                        src = pl.multiple_of(r * 2 * H, 2 * H)
                        even = pltpu.bitcast(w_v[g, pl.ds(src, H), :], U32)
                        odd = pltpu.bitcast(w_v[g, pl.ds(src + H, H), :], U32)
                        dst = pl.ds(g * per_region + r, H // 2, stride=pitch)
                        wh_s[0, dst, :] = (even & U32(0xFFFF)) | (odd << U32(16))
                        wh_s[1, dst, :] = (even >> U32(16)) | (odd & U32(0xFFFF0000))
                    return carry
                lax.fori_loop(0, per_region // 8, body, 0)
                stream.pump(1)

        def head(h, rows):
            pitch = rows // 2 + 1
            return pltpu.bitcast(wh_s[h % 2, pl.ds(h // 2 * pitch, rows // 2), :], BF16)

        front = _Stream([
            ("wm", _copy_steps(wm_hbm, wm_v, lambda r: sem_wm, 96, SMALL_SPLIT, 6), -1.5, 0.5),
            ("wq", steps_of(wq_hbm, wq_v, sem_wq), -1.0, 1.0),
            ("wuk", steps_of(wuk_hbm, wuk_v, sem_wuk), 0.0, 2.0),
            ("k0", ckv_steps(0), 1.0, 3.0),
            ("k1", ckv_steps(1), 2.0, 4.0),
            ("k2", ckv_steps(2)[:half], 3.0, 4.0),
        ])

        c_cp = pltpu.make_async_copy(c_hbm, c_v, sem_c)
        x_cp = pltpu.make_async_copy(x_hbm, x_v, sem_x)
        front.pump(4)
        c_cp.start()
        x_cp.start()
        front.pump_to(LAG)
        c_cp.wait()
        c = c_v[...].astype(F32)
        sc = (c * jax.nn.sigmoid(c)).astype(BF16)
        x_cp.wait()
        x = x_v[...].astype(F32)
        xn = _layernorm(x)
        front.pump_past("wm")
        wait(wm_hbm, wm_v, sem_wm)
        mod = []
        for i in range(6):
            mod.append(_dot(sc, wm_v[:, :, i * M:(i + 1) * M].reshape(-1, M)))
            front.pump(2)
        sa, ca, ga, sb, cb, gb = mod
        h = (xn * (1.0 + ca) + sa).astype(BF16)

        front.pump_past("wq")
        wait(wq_hbm, wq_v, sem_wq)
        split_heads(wq_v, front)
        for i in range(H):
            q_s[i] = _dot(h, head(i, M))
            front.pump(i % 2)

        front.pump_past("wuk")
        wait(wuk_hbm, wuk_v, sem_wuk)
        split_heads(wuk_v, front)
        for i in range(H):
            r = _dot_nt(q_s[i].astype(BF16), head(i, Dc)) * scale
            for t in range(n_ct):
                qa_s[t, pl.ds(i, B, stride=H), :] = r[:, t * LANES:(t + 1) * LANES]
            front.pump(i % 2)
        front.flush()

        def attend(b, stream, steps):
            r0 = b * H if isinstance(b, int) else pl.multiple_of(b * H, H)
            g0 = b * REGIONS
            per_chunk = steps // (2 * REGIONS)
            qb = jnp.concatenate(
                [qa_s[t, pl.ds(r0, H), :] for t in range(n_ct)], axis=1).astype(BF16)
            wait(ckv_hbm, ckv_v, sems.at[b], pl.ds(g0, REGIONS))
            mt = None
            for i in range(REGIONS):
                s = _dot_nt(qb, ckv_v[g0 + i])
                s_s[:, i * kc:(i + 1) * kc] = s
                for t in range(kc // LANES):
                    st = s[:, t * LANES:(t + 1) * LANES]
                    mt = st if mt is None else jnp.maximum(mt, st)
                stream.pump(per_chunk)
            m = jnp.max(mt, axis=1, keepdims=True)
            lt = None
            acc = None
            for i in range(REGIONS):
                p = jnp.exp(s_s[:, i * kc:(i + 1) * kc] - m)
                for t in range(kc // LANES):
                    pt = p[:, t * LANES:(t + 1) * LANES]
                    lt = pt if lt is None else lt + pt
                d = _dot(p.astype(BF16), ckv_v[g0 + i])
                acc = d if acc is None else acc + d
                stream.pump(per_chunk)
            ctx = acc / jnp.sum(lt, axis=1, keepdims=True)
            for t in range(n_ct):
                ctx_s[t, pl.ds(r0, H), :] = ctx[:, t * LANES:(t + 1) * LANES]

        def attn_body(b, carry):
            stream = _Stream([("a", ckv_steps(b + 2)[half:], 0.0, 1.0),
                              ("b", ckv_steps(b + 3)[:half], 0.0, 1.0)])
            attend(b, stream, ATTN_STEPS)
            stream.flush()
            return carry

        lax.fori_loop(0, B - 3, attn_body, 0)

        def w4_copies(part, rows, priority, r0=None, r1=None):
            r0 = W4_CUTS[part] if r0 is None else r0
            r1 = W4_CUTS[part + 1] if r1 is None else r1
            return [(w4_hbm, w4_v, sem_w4[part], pl.ds(r, rows), priority)
                    for r in range(r0, r1, rows)]

        mid = W4_CUTS[1] * 7 // 16
        w4_main = [[lo, hi] for lo, hi in zip(
            [cp for cps in zip(w4_copies(0, 56, LO, 0, mid), w4_copies(0, 56, LO, mid, 2 * mid))
             for cp in cps],
            w4_copies(0, 8, HI, 2 * mid), strict=True)]
        w4_last = [[lo, hi] for lo, hi in zip(
            [cp for part in range(2, len(sem_w4)) for cp in w4_copies(part, 16, LO)],
            w4_copies(1, 8, HI), strict=True)]
        wo_steps = steps_of(wo_hbm, wo_v, sem_wo)
        back = _Stream([
            ("k7", ckv_steps(B - 1)[half:], -2.0, -1.0),
            ("wuv", steps_of(wuv_hbm, wuv_v, sem_wuv), -2.0, 0.0),
            ("wo", wo_steps[:half], -1.0, 0.0),
            ("wo", wo_steps[half:], 0.0, 0.6),
            ("w3", _copy_steps(w3_hbm, w3_v, lambda r: sem_w3, 32, SMALL_SPLIT, 2), 0.0, 0.8),
            ("w4", w4_main, 0.7, 1.0),
            ("w4_last", w4_last, 1.0, 2.0),
        ])
        attend(B - 3, back, LATE_ATTN_STEPS)
        back.pump_to(LAG)
        attend(B - 2, back, LATE_ATTN_STEPS)
        back.pump_past("k7")
        attend(B - 1, back, LATE_ATTN_STEPS)

        back.pump_past("wuv")
        wait(wuv_hbm, wuv_v, sem_wuv)
        split_heads(wuv_v, back)
        for i in range(H):
            cx = jnp.concatenate(
                [ctx_s[t, pl.ds(i, B, stride=H), :] for t in range(n_ct)], axis=1).astype(BF16)
            cv_s[:, i * D:(i + 1) * D] = _dot(cx, head(i, Dc))
            back.pump(i % 2)

        back.pump_past("wo")
        wait(wo_hbm, wo_v, sem_wo)
        att = None
        k = H * D // REGIONS
        for i in range(REGIONS):
            d = _dot(cv_s[:, i * k:(i + 1) * k].astype(BF16), wo_v[i])
            att = d if att is None else att + d
            back.pump(2)
        x = x + ga * att
        h2 = _layernorm(x) * (1.0 + cb) + sb

        hn = _layernorm(h2).astype(BF16)
        back.pump_past("w3")
        wait(w3_hbm, w3_v, sem_w3)
        g = jax.nn.gelu(_dot(hn, w3_v[...].reshape(M, F)), approximate=True).astype(BF16)
        back.flush()
        y = h2
        for sem, f0, f1 in zip(sem_w4, W4_CUTS, W4_CUTS[1:]):
            wait(w4_hbm, w4_v, sem, pl.ds(f0, f1 - f0))
            y = y + _dot(g[:, f0:f1], w4_v[f0:f1, :])
        o_ref[...] = (x + gb * y).astype(o_ref.dtype)

    return kernel


@jax.jit
def pallas_adaLN_cond__compressed_kv_cla__mixer_s_mlp__decode_kernel(
    A_x: jax.Array,
    A_c_kv: jax.Array,
    A_w_q: jax.Array,
    A_w_uk: jax.Array,
    A_w_uv: jax.Array,
    A_w_o: jax.Array,
    B_x: jax.Array,
    B_w1: jax.Array,
    B_w2: jax.Array,
    B_w3: jax.Array,
    B_w4: jax.Array,
    c: jax.Array,
    w_mod: jax.Array,
):
    B, Sq, M = A_x.shape
    _, Sk, Dc = A_c_kv.shape
    _, H, D = A_w_q.shape
    F = B_w3.shape[1]
    assert Sq == 1 and D == LANES and F == W4_CUTS[-1]
    small_regions = sum(n for n, _ in SMALL_SPLIT)

    ins = (
        A_x.reshape(B, M),
        c,
        w_mod.reshape(small_regions, -1, 6 * M),
        A_w_q.reshape(REGIONS, -1, D),
        A_w_uk.reshape(REGIONS, -1, D),
        A_c_kv.reshape(B * REGIONS, Sk // REGIONS, Dc),
        A_w_uv.reshape(REGIONS, -1, D),
        A_w_o.reshape(REGIONS, -1, M),
        B_w3.reshape(small_regions, -1, F),
        B_w4,
    )
    out = pl.pallas_call(
        _make_kernel(B, H, D, M, Dc, Sk, F),
        out_shape=jax.ShapeDtypeStruct((B, M), A_x.dtype),
        in_specs=[pl.BlockSpec(memory_space=pltpu.HBM)] * len(ins),
        out_specs=pl.BlockSpec(memory_space=pltpu.VMEM),
        scratch_shapes=[
            *(pltpu.VMEM(a.shape, a.dtype) for a in ins),
            pltpu.VMEM((2, (H // 2 + 1) * (max(M, Dc) // 2 + 1), D), U32),
            pltpu.VMEM((H, B, D), F32),
            pltpu.VMEM((Dc // LANES, (B + 1) * H, LANES), F32),
            pltpu.VMEM((H, Sk), F32),
            pltpu.VMEM((Dc // LANES, (B + 1) * H, LANES), F32),
            pltpu.VMEM((B, H * D), F32),
            pltpu.SemaphoreType.DMA((B + 8 + len(W4_CUTS) - 1,)),
        ],
        compiler_params=pltpu.CompilerParams(
            vmem_limit_bytes=100 * 1024 * 1024,
            disable_bounds_checks=True,
            disable_semaphore_checks=True,
        ),
    )(*ins)
    return out.reshape(B, Sq, M)
```

```python
import jax
import jax.numpy as jnp
import numpy as np
from jax import lax
import jax.experimental.pallas as pl
import jax.experimental.pallas.tpu as pltpu

F32 = jnp.float32
BF16 = jnp.bfloat16
U32 = jnp.uint32
LANES = 128

LO, HI = 1, 0
REGIONS = 8
STEPS = 64
SPLIT = ((7, LO), (1, HI))
SMALL_SPLIT = ((3, LO), (1, HI))
LAG = 32
ATTN_STEPS = 48
LATE_ATTN_STEPS = 32
W4_CUTS = (0, 1024, 1280, 1664, 1792)


def _layernorm(x, eps=1e-5):
    d = x - jnp.mean(x, axis=-1, keepdims=True)
    return d * lax.rsqrt(jnp.mean(d * d, axis=-1, keepdims=True) + eps)


def _dot(a, b):
    return jnp.dot(a, b, preferred_element_type=F32)


def _dot_nt(a, b):
    return lax.dot_general(a, b, (((1,), (1,)), ((), ())), preferred_element_type=F32)


def _copy_steps(src, dst, sem_of, n_steps, split, col_chunks=1, g0=0):
    rows = src.shape[1] * col_chunks // n_steps
    cols = src.shape[2] // col_chunks
    assert rows * n_steps == src.shape[1] * col_chunks and cols * col_chunks == src.shape[2]
    steps = []
    for i in range(n_steps):
        r0 = i // col_chunks * rows
        slab = (pl.ds(r0, rows), pl.ds(i % col_chunks * cols, cols))
        step, g = [], 0
        for n, priority in split:
            step.append((src, dst, sem_of(r0), (pl.ds(g0 + g, n), *slab), priority))
            g += n
        steps.append(step)
    return steps


class _Stream:
    def __init__(self, spans):
        timed = [(t0 + (t1 - t0) * (i + 0.5) / len(steps), k, name, step)
                 for k, (name, steps, t0, t1) in enumerate(spans) for i, step in enumerate(steps)]
        timed.sort(key=lambda e: e[:2])
        self.steps = [e[3] for e in timed]
        self.end = {e[2]: i + 1 for i, e in enumerate(timed)}
        self.pos = 0

    def pump(self, n):
        for step in self.steps[self.pos:self.pos + n]:
            for src, dst, sem, idx, priority in step:
                pltpu.make_async_copy(src.at[idx], dst.at[idx], sem).start(priority=priority)
        self.pos = min(self.pos + n, len(self.steps))

    def pump_to(self, pos):
        self.pump(max(0, pos - self.pos))

    def pump_past(self, name):
        self.pump_to(self.end[name] + LAG)

    def flush(self):
        self.pump_to(len(self.steps))


def _make_kernel(B, H, D, M, Dc, Sk, F):
    scale = float(D) ** -0.5
    kc = Sk // REGIONS
    n_ct = Dc // LANES
    half = STEPS // 2

    def kernel(x_hbm, c_hbm, wm_hbm, wq_hbm, wuk_hbm, ckv_hbm, wuv_hbm, wo_hbm, w3_hbm, w4_hbm,
               o_ref,
               x_v, c_v, wm_v, wq_v, wuk_v, ckv_v, wuv_v, wo_v, w3_v, w4_v,
               wh_s, q_s, qa_s, s_s, ctx_s, cv_s, sems):
        (sem_x, sem_c, sem_wm, sem_wq, sem_wuk, sem_wuv, sem_wo, sem_w3, *sem_w4) = (
            sems.at[i] for i in range(B, sems.shape[0]))

        def steps_of(src, dst, sem):
            return _copy_steps(src, dst, lambda r: sem, STEPS, SPLIT)

        def ckv_steps(b):
            return _copy_steps(ckv_hbm, ckv_v, lambda r: sems.at[b], STEPS, SPLIT, g0=b * REGIONS)

        def wait(src, dst, sem, idx=...):
            pltpu.make_async_copy(src.at[idx], dst.at[idx], sem).wait()

        def split_heads(w_v, stream):
            per_region = w_v.shape[1] // (2 * H)
            pitch = REGIONS * per_region + 1
            low, high, shift = np.uint32(0xFFFF), np.uint32(0xFFFF0000), np.uint32(16)
            for g in range(REGIONS):
                def body(i, carry, g=g):
                    for t in range(8):
                        r = i * 8 + t
                        src = pl.multiple_of(r * 2 * H, 2 * H)
                        even = pltpu.bitcast(w_v[g, pl.ds(src, H), :], U32)
                        odd = pltpu.bitcast(w_v[g, pl.ds(src + H, H), :], U32)
                        dst = pl.ds(g * per_region + r, H // 2, stride=pitch)
                        wh_s[0, dst, :] = (even & low) | (odd << shift)
                        wh_s[1, dst, :] = (even >> shift) | (odd & high)
                    return carry
                lax.fori_loop(0, per_region // 8, body, 0)
                stream.pump(1)

        def head(h, rows):
            pitch = rows // 2 + 1
            return pltpu.bitcast(wh_s[h % 2, pl.ds(h // 2 * pitch, rows // 2), :], BF16)

        front = _Stream([
            ("wm", _copy_steps(wm_hbm, wm_v, lambda r: sem_wm, 96, SMALL_SPLIT, 6), -1.5, 0.5),
            ("wq", steps_of(wq_hbm, wq_v, sem_wq), -1.0, 1.0),
            ("wuk", steps_of(wuk_hbm, wuk_v, sem_wuk), 0.0, 2.0),
            ("k0", ckv_steps(0), 1.0, 3.0),
            ("k1", ckv_steps(1), 2.0, 4.0),
            ("k2", ckv_steps(2)[:half], 3.0, 4.0),
        ])

        c_cp = pltpu.make_async_copy(c_hbm, c_v, sem_c)
        x_cp = pltpu.make_async_copy(x_hbm, x_v, sem_x)
        front.pump(4)
        c_cp.start()
        x_cp.start()
        front.pump_to(LAG)
        c_cp.wait()
        c = c_v[...].astype(F32)
        sc = (c * jax.nn.sigmoid(c)).astype(BF16)
        x_cp.wait()
        x = x_v[...].astype(F32)
        xn = _layernorm(x)
        front.pump_past("wm")
        wait(wm_hbm, wm_v, sem_wm)
        mod = []
        for i in range(6):
            mod.append(_dot(sc, wm_v[:, :, i * M:(i + 1) * M].reshape(-1, M)))
            front.pump(2)
        sa, ca, ga, sb, cb, gb = mod
        h = (xn * (1.0 + ca) + sa).astype(BF16)

        front.pump_past("wq")
        wait(wq_hbm, wq_v, sem_wq)
        split_heads(wq_v, front)
        for i in range(H):
            q_s[i] = _dot(h, head(i, M))
            front.pump(i % 2)

        front.pump_past("wuk")
        wait(wuk_hbm, wuk_v, sem_wuk)
        split_heads(wuk_v, front)
        for i in range(H):
            r = _dot_nt(q_s[i].astype(BF16), head(i, Dc)) * scale
            for t in range(n_ct):
                qa_s[t, pl.ds(i, B, stride=H), :] = r[:, t * LANES:(t + 1) * LANES]
            front.pump(i % 2)
        front.flush()

        def attend(b, stream, steps):
            r0 = b * H if isinstance(b, int) else pl.multiple_of(b * H, H)
            g0 = b * REGIONS
            per_chunk = steps // (2 * REGIONS)
            qb = jnp.concatenate(
                [qa_s[t, pl.ds(r0, H), :] for t in range(n_ct)], axis=1).astype(BF16)
            wait(ckv_hbm, ckv_v, sems.at[b], pl.ds(g0, REGIONS))
            mt = None
            for i in range(REGIONS):
                s = _dot_nt(qb, ckv_v[g0 + i])
                s_s[:, i * kc:(i + 1) * kc] = s
                for t in range(kc // LANES):
                    st = s[:, t * LANES:(t + 1) * LANES]
                    mt = st if mt is None else jnp.maximum(mt, st)
                stream.pump(per_chunk)
            m = jnp.max(mt, axis=1, keepdims=True)
            lt = None
            acc = None
            for i in range(REGIONS):
                p = jnp.exp(s_s[:, i * kc:(i + 1) * kc] - m)
                for t in range(kc // LANES):
                    pt = p[:, t * LANES:(t + 1) * LANES]
                    lt = pt if lt is None else lt + pt
                d = _dot(p.astype(BF16), ckv_v[g0 + i])
                acc = d if acc is None else acc + d
                stream.pump(per_chunk)
            ctx = acc / jnp.sum(lt, axis=1, keepdims=True)
            for t in range(n_ct):
                ctx_s[t, pl.ds(r0, H), :] = ctx[:, t * LANES:(t + 1) * LANES]

        def attn_body(b, carry):
            stream = _Stream([("a", ckv_steps(b + 2)[half:], 0.0, 1.0),
                              ("b", ckv_steps(b + 3)[:half], 0.0, 1.0)])
            attend(b, stream, ATTN_STEPS)
            stream.flush()
            return carry

        lax.fori_loop(0, B - 3, attn_body, 0)

        def w4_copies(part, rows, priority, r0=None, r1=None):
            r0 = W4_CUTS[part] if r0 is None else r0
            r1 = W4_CUTS[part + 1] if r1 is None else r1
            return [(w4_hbm, w4_v, sem_w4[part], pl.ds(r, rows), priority)
                    for r in range(r0, r1, rows)]

        mid = W4_CUTS[1] * 7 // 16
        w4_main = [[lo, hi] for lo, hi in zip(
            [cp for cps in zip(w4_copies(0, 56, LO, 0, mid), w4_copies(0, 56, LO, mid, 2 * mid))
             for cp in cps],
            w4_copies(0, 8, HI, 2 * mid), strict=True)]
        w4_last = [[lo, hi] for lo, hi in zip(
            [cp for part in range(2, len(sem_w4)) for cp in w4_copies(part, 16, LO)],
            w4_copies(1, 8, HI), strict=True)]
        wo_steps = steps_of(wo_hbm, wo_v, sem_wo)
        back = _Stream([
            ("k7", ckv_steps(B - 1)[half:], -2.0, -1.0),
            ("wuv", steps_of(wuv_hbm, wuv_v, sem_wuv), -2.0, 0.0),
            ("wo", wo_steps[:half], -1.0, 0.0),
            ("wo", wo_steps[half:], 0.0, 0.6),
            ("w3", _copy_steps(w3_hbm, w3_v, lambda r: sem_w3, 32, SMALL_SPLIT, 2), 0.0, 0.8),
            ("w4", w4_main, 0.7, 1.0),
            ("w4_last", w4_last, 1.0, 2.0),
        ])
        attend(B - 3, back, LATE_ATTN_STEPS)
        back.pump_to(LAG)
        attend(B - 2, back, LATE_ATTN_STEPS)
        back.pump_past("k7")
        attend(B - 1, back, LATE_ATTN_STEPS)

        back.pump_past("wuv")
        wait(wuv_hbm, wuv_v, sem_wuv)
        split_heads(wuv_v, back)
        for i in range(H):
            cx = jnp.concatenate(
                [ctx_s[t, pl.ds(i, B, stride=H), :] for t in range(n_ct)], axis=1).astype(BF16)
            cv_s[:, i * D:(i + 1) * D] = _dot(cx, head(i, Dc))
            back.pump(i % 2)

        back.pump_past("wo")
        wait(wo_hbm, wo_v, sem_wo)
        att = None
        k = H * D // REGIONS
        for i in range(REGIONS):
            d = _dot(cv_s[:, i * k:(i + 1) * k].astype(BF16), wo_v[i])
            att = d if att is None else att + d
            back.pump(2)
        x = x + ga * att
        h2 = _layernorm(x) * (1.0 + cb) + sb

        hn = _layernorm(h2).astype(BF16)
        back.pump_past("w3")
        back.pump(4)
        wait(w3_hbm, w3_v, sem_w3)
        g = jax.nn.gelu(_dot(hn, w3_v[...].reshape(M, F)), approximate=True).astype(BF16)
        back.flush()
        y = h2
        for sem, f0, f1 in zip(sem_w4, W4_CUTS, W4_CUTS[1:]):
            wait(w4_hbm, w4_v, sem, pl.ds(f0, f1 - f0))
            y = y + _dot(g[:, f0:f1], w4_v[f0:f1, :])
        o_ref[...] = (x + gb * y).astype(o_ref.dtype)

    return kernel


@jax.jit
def pallas_adaLN_cond__compressed_kv_cla__mixer_s_mlp__decode_kernel(
    A_x: jax.Array,
    A_c_kv: jax.Array,
    A_w_q: jax.Array,
    A_w_uk: jax.Array,
    A_w_uv: jax.Array,
    A_w_o: jax.Array,
    B_x: jax.Array,
    B_w1: jax.Array,
    B_w2: jax.Array,
    B_w3: jax.Array,
    B_w4: jax.Array,
    c: jax.Array,
    w_mod: jax.Array,
):
    B, Sq, M = A_x.shape
    _, Sk, Dc = A_c_kv.shape
    _, H, D = A_w_q.shape
    F = B_w3.shape[1]
    assert Sq == 1 and D == LANES and F == W4_CUTS[-1]
    small_regions = sum(n for n, _ in SMALL_SPLIT)

    ins = (
        A_x.reshape(B, M),
        c,
        w_mod.reshape(small_regions, -1, 6 * M),
        A_w_q.reshape(REGIONS, -1, D),
        A_w_uk.reshape(REGIONS, -1, D),
        A_c_kv.reshape(B * REGIONS, Sk // REGIONS, Dc),
        A_w_uv.reshape(REGIONS, -1, D),
        A_w_o.reshape(REGIONS, -1, M),
        B_w3.reshape(small_regions, -1, F),
        B_w4,
    )
    out = pl.pallas_call(
        _make_kernel(B, H, D, M, Dc, Sk, F),
        out_shape=jax.ShapeDtypeStruct((B, M), A_x.dtype),
        in_specs=[pl.BlockSpec(memory_space=pltpu.HBM)] * len(ins),
        out_specs=pl.BlockSpec(memory_space=pltpu.VMEM),
        scratch_shapes=[
            *(pltpu.VMEM(a.shape, a.dtype) for a in ins),
            pltpu.VMEM((2, (H // 2 + 1) * (max(M, Dc) // 2 + 1), D), U32),
            pltpu.VMEM((H, B, D), F32),
            pltpu.VMEM((Dc // LANES, (B + 1) * H, LANES), F32),
            pltpu.VMEM((H, Sk), F32),
            pltpu.VMEM((Dc // LANES, (B + 1) * H, LANES), F32),
            pltpu.VMEM((B, H * D), F32),
            pltpu.SemaphoreType.DMA((B + 8 + len(W4_CUTS) - 1,)),
        ],
        compiler_params=pltpu.CompilerParams(
            vmem_limit_bytes=100 * 1024 * 1024,
            disable_bounds_checks=True,
            disable_semaphore_checks=True,
        ),
    )(*ins)
    return out.reshape(B, Sq, M)
```
